```python
import jax
import jax.numpy as jnp

def _softmax(x, axis=-1):
    return jax.nn.softmax(x, axis=axis)
def _gelu(x):
    return jax.nn.gelu(x, approximate=True)
def _silu(x):
    return jax.nn.silu(x)
def _sigmoid(x):
    return jax.nn.sigmoid(x)
def _layernorm(x, axis=-1, eps=1e-5):
    m = jnp.mean(x, axis=axis, keepdims=True)
    v = jnp.var(x, axis=axis, keepdims=True)
    return (x - m) / jnp.sqrt(v + eps)
def _scatter_add(tgt, idx, src, axis=0):
    return tgt.at[idx].add(src)
def _segment_sum(src, seg, n):
    return jax.ops.segment_sum(src, seg, n)
class _Rng:
    def __init__(self, key):
        self._k = key
    def _next(self):
        self._k, sub = jax.random.split(self._k)
        return sub
    def normal(self, shape):
        return jax.random.normal(self._next(), shape, dtype=jnp.bfloat16)
    def randint(self, lo, hi, shape):
        return jax.random.randint(self._next(), shape, lo, hi, dtype=jnp.int32)
    def uniform(self, shape, lo=0.0, hi=1.0):
        return jax.random.uniform(self._next(), shape, jnp.bfloat16, lo, hi)
    def permutation(self, n):
        return jax.random.permutation(self._next(), n)


kernel_name = 'interleave_layers__gqa_block_cached__sliding_block_cached__decode'

def _fwd_setup_inputs():
    _rng = _Rng(jax.random.key(int.from_bytes(__import__("os").urandom(4), "little")))
    _w = (lambda a: (lambda t: t.astype(jnp.bfloat16) if jnp.issubdtype(t.dtype, jnp.floating) else t)(jnp.asarray(a)))
    def _A_setup():
        B, Sq, D = 1, 1, 640
        Hq, Hkv, Sk, Dh = 32, 32, 8192, 128
        assert Hq % Hkv == 0, (Hq, Hkv)
        return {
            "x": _w((lambda *s: _rng.normal(s) * 0.05)(B, Sq, D)),
            "k_cache": _w((lambda *s: _rng.normal(s) * 0.05)(B, Hkv, Sk, Dh)),
            "v_cache": _w((lambda *s: _rng.normal(s) * 0.05)(B, Hkv, Sk, Dh)),
            "wq": _w((lambda *s: _rng.normal(s) * 0.05)(D, Hq * Dh) * (D ** -0.5)),
            "wo": _w((lambda *s: _rng.normal(s) * 0.05)(Hq * Dh, D) * ((Hq * Dh) ** -0.5)),
        }
    _A_in = _A_setup()

    def _B_setup():
        B, Sq, D = 1, 1, 640
        Hq, Hkv, Sk, Dh = 32, 32, 8192, 128
        assert Hq % Hkv == 0, (Hq, Hkv)
        return {
            "x": _w((lambda *s: _rng.normal(s) * 0.05)(B, Sq, D)),
            "k_cache": _w((lambda *s: _rng.normal(s) * 0.05)(B, Hkv, Sk, Dh)),
            "v_cache": _w((lambda *s: _rng.normal(s) * 0.05)(B, Hkv, Sk, Dh)),
            "wq": _w((lambda *s: _rng.normal(s) * 0.05)(D, Hq * Dh) * (D ** -0.5)),
            "wo": _w((lambda *s: _rng.normal(s) * 0.05)(Hq * Dh, D) * ((Hq * Dh) ** -0.5)),
        }
    _B_in = _B_setup()

    return {
        "A_x": _A_in["x"],
        "A_k_cache": _A_in["k_cache"],
        "A_v_cache": _A_in["v_cache"],
        "A_wq": _A_in["wq"],
        "A_wo": _A_in["wo"],
        "B_x": _B_in["x"],
        "B_k_cache": _B_in["k_cache"],
        "B_v_cache": _B_in["v_cache"],
        "B_wq": _B_in["wq"],
        "B_wo": _B_in["wo"],
    }

def _fwd_reference(A_x, A_k_cache, A_v_cache, A_wq, A_wo, B_x, B_k_cache, B_v_cache, B_wq, B_wo):
    def _A_ref(x, k_cache, v_cache, wq, wo):
        B, Sq, D = x.shape
        Hq, Dh = 32, 128
        Hkv = k_cache.shape[1]
        rep = Hq // Hkv
        q = (lambda x, *d: x.transpose(*d))((x @ wq).reshape(B, Sq, Hq, Dh), 0, 2, 1, 3)
        k = jnp.repeat(k_cache, rep, axis=1)
        v = jnp.repeat(v_cache, rep, axis=1)
        scores = jnp.einsum("bhqd,bhkd->bhqk", q, k) * (Dh ** -0.5)
        p = _softmax(scores, axis=-1)
        o = jnp.einsum("bhqk,bhkd->bhqd", p, v)
        return (lambda x, *d: x.transpose(*d))(o, 0, 2, 1, 3).reshape(B, Sq, Hq * Dh) @ wo

    def _B_ref(x, k_cache, v_cache, wq, wo):
        B, Sq, D = x.shape
        Hq, Dh = 32, 128
        Hkv, Sk = k_cache.shape[1], k_cache.shape[2]
        W = min(4096, max(256, Sk // 4))
        rep = Hq // Hkv
        q = (lambda x, *d: x.transpose(*d))((x @ wq).reshape(B, Sq, Hq, Dh), 0, 2, 1, 3)
        k = jnp.repeat(k_cache[:, :, Sk - W:, :], rep, axis=1)
        v = jnp.repeat(v_cache[:, :, Sk - W:, :], rep, axis=1)
        scores = jnp.einsum("bhqd,bhkd->bhqk", q, k) * (Dh ** -0.5)
        p = _softmax(scores, axis=-1)
        o = jnp.einsum("bhqk,bhkd->bhqd", p, v)
        return (lambda x, *d: x.transpose(*d))(o, 0, 2, 1, 3).reshape(B, Sq, Hq * Dh) @ wo

    x = A_x
    x = x + _A_ref(_layernorm(x, axis=-1), A_k_cache, A_v_cache, A_wq, A_wo)
    x = x + _B_ref(_layernorm(x, axis=-1), B_k_cache, B_v_cache, B_wq, B_wo)
    x = x + _A_ref(_layernorm(x, axis=-1), A_k_cache, A_v_cache, A_wq, A_wo)
    x = x + _B_ref(_layernorm(x, axis=-1), B_k_cache, B_v_cache, B_wq, B_wo)
    return x


def setup_inputs():
    _inp = _fwd_setup_inputs()
    _gk = jax.random.fold_in(jax.random.key(int.from_bytes(__import__("os").urandom(4), "little")), 2**31 - 1)
    _shapes = [[1, 1, 640]]
    _dtypes = ['bfloat16']
    _gks = jax.random.split(_gk, len(_shapes))
    _gs = [jax.random.normal(k, s, dtype=jnp.dtype(d)) * 0.05 for k, s, d in zip(_gks, _shapes, _dtypes)]
    _inp["grad_out"] = _gs[0]
    return _inp

def reference(A_x, A_k_cache, A_v_cache, A_wq, A_wo, B_k_cache, B_v_cache, B_wq, B_wo, B_x, grad_out):
    _const = dict(B_x=B_x)
    def _f(*_d):
        return _fwd_reference(**{'A_x': _d[0], 'A_k_cache': _d[1], 'A_v_cache': _d[2], 'A_wq': _d[3], 'A_wo': _d[4], 'B_k_cache': _d[5], 'B_v_cache': _d[6], 'B_wq': _d[7], 'B_wo': _d[8], **_const})
    _out, _vjp = jax.vjp(_f, A_x, A_k_cache, A_v_cache, A_wq, A_wo, B_k_cache, B_v_cache, B_wq, B_wo)
    _grads = _vjp(grad_out)
    _out0 = jnp.asarray(_out)
    return (_out0, *[jnp.asarray(_g) for _g in _grads])
```

```python
import jax
import jax.numpy as jnp
from jax import lax
import jax.experimental.pallas as pl
import jax.experimental.pallas.tpu as pltpu

F32 = jnp.float32
BF16 = jnp.bfloat16

D = 640
H = 32
DH = 128
SK = 8192
WIN = 2048
G = 8
NG = H // G
GW = G * DH
EPS = 1e-5
SCALE = DH ** -0.5

NSLOT = 5
CH = 256
OC = 512
WR = 128
ZR = 64
M3_ROW = NG * (SK // DH) * 16

NN = (((1,), (0,)), ((), ()))
NT = (((1,), (1,)), ((), ()))
TN = (((0,), (0,)), ((), ()))


def _dot(a, b, dims):
    return lax.dot_general(a, b, dims, preferred_element_type=F32)


def _row_ids():
    return lax.broadcasted_iota(jnp.int32, (G, DH), 0)


def _only_row(x, r):
    return jnp.where(_row_ids() == r, x, 0.0)


def _block_diag(x):
    return jnp.concatenate([_only_row(x, r) for r in range(G)], axis=1)


def _compact(y):
    out = y[:, :DH]
    rows = _row_ids()
    for r in range(1, G):
        out = jnp.where(rows == r, y[:, r * DH:(r + 1) * DH], out)
    return out


def _pair(a, b, r):
    return jnp.concatenate([_only_row(a, r), _only_row(b, r)], axis=0).astype(BF16)


def _layernorm(x):
    mean = jnp.mean(x, axis=-1, keepdims=True)
    xc = x - mean
    var = jnp.mean(xc * xc, axis=-1, keepdims=True)
    rstd = 1.0 / jnp.sqrt(var + EPS)
    return xc * rstd, rstd


def _layernorm_bwd(dn, n, rstd):
    return rstd * (dn - jnp.mean(dn, axis=-1, keepdims=True)
                   - n * jnp.mean(dn * n, axis=-1, keepdims=True))


def _softmax(s):
    e = jnp.exp(s - jnp.max(s, axis=-1, keepdims=True))
    return e * (1.0 / jnp.sum(e, axis=-1, keepdims=True))


Q1, Q2, Q3, Q4, O1, O2, O3, O4, DO1, DO2, DO3, DO4, DQ1, DQ2, DQ3, DQ4 = range(16)


def _kernel(x_hbm, ka_hbm, va_hbm, wqa_hbm, woa_hbm, kb_hbm, vb_hbm, wqb_hbm, wob_hbm, g_hbm,
            out_hbm, dx_hbm, dka_hbm, dva_hbm, dwqa_hbm, dwoa_hbm, dkb_hbm, dvb_hbm, dwqb_hbm, dwob_hbm,
            va, kb, vb, ka, wqa, woa, wqb, wob, m1, tab, pbuf, zbuf, xin, xout, one,
            sem_ka, sem_va, sem_b, sem_w, sem_x, sem_z, sem_o):

    one[0] = 1

    def section(f):
        pl.when(one[0] > 0)(f)

    def grp(g):
        return pl.ds(pl.multiple_of(g * G, G), G)

    def ka_copy(head, slot):
        return pltpu.make_async_copy(ka_hbm.at[head], ka.at[slot], sem_ka.at[slot])

    def va_copy(head):
        return pltpu.make_async_copy(va_hbm.at[head], va.at[head], sem_va.at[head % NSLOT])

    def b_copy(which, g):
        src, dst = ((kb_hbm, kb), (vb_hbm, vb))[which]
        return pltpu.make_async_copy(src.at[pl.ds(g * G, G), pl.ds(SK - WIN, WIN), :],
                                     dst.at[pl.ds(g * G, G)], sem_b.at[which, g])

    def wq_copies(src, dst, s):
        return [pltpu.make_async_copy(src.at[:, pl.ds(g * GW, GW)], dst.at[g], sem_w.at[s])
                for g in range(NG)]

    def wo_copy(src, dst, s):
        return pltpu.make_async_copy(src, dst, sem_w.at[s])

    nzj = (SK - WIN) // ZR
    nz = 2 * NG * nzj

    def zero_start(lo, hi):
        def body(i, c):
            g, j = i // nzj, i % nzj
            for dst in (dkb_hbm, dvb_hbm):
                pltpu.make_async_copy(
                    zbuf, dst.at[grp(g), pl.ds(pl.multiple_of(j * ZR, ZR), ZR), :], sem_z.at[0]).start()
            return c
        lax.fori_loop(lo // 2, hi // 2, body, 0)

    def zero_wait(lo, hi):
        def body(i, c):
            pltpu.make_async_copy(zbuf, dkb_hbm.at[pl.ds(0, G), pl.ds(0, ZR), :], sem_z.at[0]).wait()
            return c
        lax.fori_loop(lo, hi, body, 0)

    def proj_in(vec, w, dims, dst):
        vb16 = vec.astype(BF16)

        def body(g, c):
            wg = w[g] if dims is NN else w[pl.ds(pl.multiple_of(g * GW, GW), GW), :]
            tab[dst, grp(g), :] = _compact(_dot(vb16, wg, dims))
            return c
        lax.fori_loop(0, NG, body, 0)

    def proj_out(src, w, dims):
        def body(g, acc):
            wg = w[g] if dims is NT else w[pl.ds(pl.multiple_of(g * GW, GW), GW), :]
            return acc + _dot(_block_diag(tab[src, grp(g), :]).astype(BF16), wg, dims)
        acc = lax.fori_loop(0, NG, body, jnp.zeros((G, D), F32))
        return jnp.broadcast_to(jnp.sum(acc, axis=0, keepdims=True), (G, D))

    def head_row(t, head):
        return jnp.broadcast_to(tab[t, pl.ds(head, 1), :], (G, DH))

    def a_probs(q, slot):
        qb = q.astype(BF16)
        s = jnp.concatenate(
            [_dot(qb, ka[slot, pl.ds(c * CH, CH), :], NT) for c in range(SK // CH)], axis=1)
        p = _softmax(s * SCALE)
        for c in range(SK // CH):
            pbuf[c] = p[:, c * CH:(c + 1) * CH]

    def a_values(slot, head):
        acc = jnp.zeros((DH + 16, DH), F32)
        ksum = jnp.zeros((DH, DH), F32)
        for c in range(SK // CH):
            rows = pl.ds(c * CH, CH)
            pc = pbuf[c]
            kp = ka[slot, rows, :].T.astype(F32) * pc[0:1, :]
            for t in range(CH // DH):
                ksum = ksum + kp[:, t * DH:(t + 1) * DH]
            lhs = jnp.concatenate([kp, pc, pc], axis=0).astype(BF16)
            acc = acc + _dot(lhs, va[head, rows, :], NN)
        o = acc[DH:DH + 1, :]
        kbar = jnp.sum(ksum, axis=1, keepdims=True)
        return o, (acc[:DH, :] - kbar * o).astype(BF16)

    def apply_m(m_of_head, src, dst):
        def body(g, c):
            do = tab[src, grp(g), :]
            dq = jnp.zeros((G, DH), F32)
            for r in range(G):
                dq = dq + _dot(_only_row(do, r).astype(BF16), m_of_head(g * G + r), NT)
            tab[dst, grp(g), :] = dq * SCALE
            return c
        lax.fori_loop(0, NG, body, 0)

    def park_load(slot, tile0, n):
        rows = ka[slot, pl.ds(pl.multiple_of(tile0 * 16, 16), n * 16), :]
        return jnp.concatenate([rows[t * 16:(t + 1) * 16, :] for t in range(n)], axis=1)

    def park_store(slot, tile0, val):
        n = val.shape[1] // DH
        ka[slot, pl.ds(pl.multiple_of(tile0 * 16, 16), n * 16), :] = jnp.concatenate(
            [val[:, t * DH:(t + 1) * DH] for t in range(n)], axis=0)

    def outer_rhs(do_a, do_b, q_a, q_b):
        zero = jnp.zeros((16, DH), BF16)
        cols = []
        for r in range(G):
            cols.append(jnp.concatenate([_pair(do_a, do_b, r), zero], axis=0))
            cols.append(jnp.concatenate([zero, _pair(q_a, q_b, r)], axis=0))
        return cols

    x_copy = pltpu.make_async_copy(x_hbm, xin.at[0], sem_x.at[0])
    g_copy = pltpu.make_async_copy(g_hbm, xin.at[1], sem_x.at[1])
    x_copy.start()
    for cp in wq_copies(wqa_hbm, wqa, 0):
        cp.start()
    g_copy.start()
    first_slot = (NSLOT - H % NSLOT) % NSLOT
    for h in range(NSLOT):
        ka_copy(h, (h + first_slot) % NSLOT).start()
        va_copy(h).start()
    zbuf[...] = jnp.zeros(zbuf.shape, BF16)

    x_copy.wait()
    x0 = jnp.broadcast_to(xin[0].astype(F32), (G, D))
    n1, rstd1 = _layernorm(x0)
    for cp in wq_copies(wqa_hbm, wqa, 0):
        cp.wait()
    proj_in(n1, wqa, NN, Q1)

    late = ([[wo_copy(woa_hbm, woa, 1)] + wq_copies(wqb_hbm, wqb, 2)]
            + [[b_copy(0, g), b_copy(1, g)] for g in range(NG)])
    late[NSLOT - 1] = late[NSLOT - 1] + [wo_copy(wob_hbm, wob, 3)]

    def layer1(h, c):
        slot = (h + first_slot) % NSLOT
        ka_copy(h, slot).wait()
        a_probs(head_row(Q1, h), slot)
        va_copy(h).wait()

        @section
        def _():
            o, m = a_values(slot, h)
            m1[h] = m
            tab[O1, pl.ds(h, 1), :] = o

        @pl.when(h + NSLOT < H)
        def _():
            ka_copy(h + NSLOT, slot).start()
            va_copy(h + NSLOT).start()
        for k, cps in enumerate(late):
            @pl.when(h == H - NSLOT + k)
            def _():
                for cp in cps:
                    cp.start()
        return c
    lax.fori_loop(0, H, layer1, 0)

    wo_copy(woa_hbm, woa, 1).wait()
    x1 = x0 + proj_out(O1, woa, NN)
    n2, rstd2 = _layernorm(x1)
    for cp in wq_copies(wqb_hbm, wqb, 2):
        cp.wait()
    proj_in(n2, wqb, NN, Q2)

    def b_scores(lhs_of_row, ref, g):
        s = _dot(lhs_of_row(0), ref[g * G], NT)
        for r in range(1, G):
            s = s + _dot(lhs_of_row(r), ref[g * G + r], NT)
        return s

    def b_mix(p, ref, g):
        pb = p.astype(BF16)
        out = _dot(pb, ref[g * G], NN)
        rows = _row_ids()
        for r in range(1, G):
            out = jnp.where(rows == r, _dot(pb, ref[g * G + r], NN), out)
        return out

    def layer2(g, c):
        b_copy(0, g).wait()
        q = tab[Q2, grp(g), :]
        p = _softmax(b_scores(lambda r: _only_row(q, r).astype(BF16), kb, g) * SCALE)
        b_copy(1, g).wait()
        tab[O2, grp(g), :] = b_mix(p, vb, g)
        return c
    lax.fori_loop(0, NG, layer2, 0)

    wo_copy(wob_hbm, wob, 3).wait()
    z0 = 128
    zero_start(0, 64)
    x2 = x1 + proj_out(O2, wob, NN)
    n3, rstd3 = _layernorm(x2)
    proj_in(n3, wqa, NN, Q3)

    ring = NSLOT - 1

    def layer3(i, c):
        head = (i + H - NSLOT) % H
        slot = jnp.where(i == 0, 0, 1 + (i + ring - 1) % ring)

        @pl.when(i >= NSLOT)
        def _():
            ka_copy(head, slot).wait()

        @pl.when(i == H - 1)
        def _():
            zero_start(z0, z0 + 64)

        rows = _row_ids()
        q = jnp.where(rows < G // 2, head_row(Q3, head), head_row(Q1, head))
        a_probs(q, slot)

        @section
        def _():
            o, m = a_values(slot, head)
            ka[0, pl.ds(pl.multiple_of(M3_ROW + head * DH, DH), DH), :] = m
            tab[O3, pl.ds(head, 1), :] = o

        @section
        def _():
            g, r = head // G, head % G
            mine = lax.broadcasted_iota(jnp.int32, (16, CH), 0) % G == r
            for cc in range(SK // CH):
                tile0 = g * (SK // DH) + cc * (CH // DH)
                pc = pbuf[cc]
                new = jnp.concatenate([jnp.broadcast_to(pc[0:1, :], (G, CH)),
                                       jnp.broadcast_to(pc[G // 2:G // 2 + 1, :], (G, CH))], axis=0)
                old = park_load(0, tile0, CH // DH).astype(F32)
                park_store(0, tile0, jnp.where(mine, new, old).astype(BF16))

        @pl.when(i == 1)
        def _():
            zero_start(64, z0)

        @pl.when(i == NSLOT - 1)
        def _():
            zero_wait(0, z0)
            for k in range(ring):
                ka_copy(k, 1 + k).start()

        @pl.when(jnp.logical_and(i >= NSLOT, i + ring < H))
        def _():
            ka_copy(head + ring, slot).start()
        return c
    lax.fori_loop(0, H, layer3, 0)

    zpos = z0 + 64

    def zero_more(n):
        nonlocal zpos
        n = min(n, nz - zpos)
        if n:
            zero_start(zpos, zpos + n)
        zpos += n

    x3 = x2 + proj_out(O3, woa, NN)
    n4, rstd4 = _layernorm(x3)
    proj_in(n4, wqb, NN, Q4)
    zero_more(32)
    g_copy.wait()
    g4 = jnp.broadcast_to(xin[1].astype(F32), (G, D))
    proj_in(g4, wob, NT, DO4)
    zero_more(16)

    nbt = WIN // DH

    def delta(o, do, g):
        return jnp.sum(tab[o, grp(g), :] * tab[do, grp(g), :], axis=1, keepdims=True)

    def layer4(g, c):
        q4, q2 = tab[Q4, grp(g), :], tab[Q2, grp(g), :]
        p = _softmax(b_scores(lambda r: _pair(q4, q2, r), kb, g) * SCALE)
        park_store(1, g * nbt, p.astype(BF16))
        p4 = p[:G, :]
        tab[O4, grp(g), :] = b_mix(p4, vb, g)
        do = tab[DO4, grp(g), :]
        dp = b_scores(lambda r: _only_row(do, r).astype(BF16), vb, g)
        ds = p4 * (dp - delta(O4, DO4, g)) * SCALE
        park_store(1, (NG + g) * nbt, jnp.concatenate([ds, ds], axis=0).astype(BF16))
        tab[DQ4, grp(g), :] = b_mix(ds, kb, g)
        zero_start(zpos + g * 32, zpos + (g + 1) * 32)
        return c
    lax.fori_loop(0, NG, layer4, 0)
    zpos += NG * 32

    x4 = x3 + proj_out(O4, wob, NN)
    xout[0] = x4[0:1, :].astype(BF16)
    out_copy = pltpu.make_async_copy(xout.at[0], out_hbm, sem_x.at[0])
    out_copy.start()
    g3 = g4 + _layernorm_bwd(proj_out(DQ4, wqb, NT), n4, rstd4)
    zero_more(32)

    proj_in(g3, woa, NT, DO3)
    apply_m(lambda h: ka[0, pl.ds(pl.multiple_of(M3_ROW + h * DH, DH), DH), :], DO3, DQ3)
    g2 = g3 + _layernorm_bwd(proj_out(DQ3, wqa, NT), n3, rstd3)
    zero_more(32)

    proj_in(g2, wob, NT, DO2)

    def layer2_bwd(g, c):
        do = tab[DO2, grp(g), :]
        dp = b_scores(lambda r: _only_row(do, r).astype(BF16), vb, g)
        p2 = park_load(1, g * nbt, nbt).astype(F32)[G:, :]
        ds = p2 * (dp - delta(O2, DO2, g)) * SCALE
        ds4 = park_load(1, (NG + g) * nbt, nbt).astype(F32)[:G, :]
        park_store(1, (NG + g) * nbt, jnp.concatenate([ds4, ds], axis=0).astype(BF16))
        tab[DQ2, grp(g), :] = b_mix(ds, kb, g)
        zero_start(zpos + g * 16, zpos + (g + 1) * 16)
        return c
    lax.fori_loop(0, NG, layer2_bwd, 0)
    zpos += NG * 16
    g1 = g2 + _layernorm_bwd(proj_out(DQ2, wqb, NT), n2, rstd2)
    zero_more(32)

    proj_in(g1, woa, NT, DO1)
    apply_m(lambda h: m1[h], DO1, DQ1)
    g0 = g1 + _layernorm_bwd(proj_out(DQ1, wqa, NT), n1, rstd1)
    xout[1] = g0[0:1, :].astype(BF16)
    dx_copy = pltpu.make_async_copy(xout.at[1], dx_hbm, sem_x.at[1])
    dx_copy.start()
    zero_more(32)

    def weight_grads(wq, wo, na, nb, dqa, dqb, oa, ob, ga, gb):
        ns = jnp.concatenate([na, nb], axis=0).astype(BF16)
        gs = jnp.concatenate([ga, gb], axis=0).astype(BF16)

        def body(g, c):
            dq = jnp.concatenate([_block_diag(tab[dqa, grp(g), :]),
                                  _block_diag(tab[dqb, grp(g), :])], axis=0).astype(BF16)
            o = jnp.concatenate([_block_diag(tab[oa, grp(g), :]),
                                 _block_diag(tab[ob, grp(g), :])], axis=0).astype(BF16)
            for r in range(G):
                cols = slice(r * DH, (r + 1) * DH)
                wq[g, :, cols] = _dot(ns, dq[:, cols], TN).astype(BF16)
                wo[pl.ds(pl.multiple_of(g * GW + r * DH, DH), DH), :] = _dot(o[:, cols], gs, TN).astype(BF16)
            return c
        lax.fori_loop(0, NG, body, 0)

    weight_grads(wqb, wob, n4, n2, DQ4, DQ2, O4, O2, g4, g2)
    zero_more(48)
    weight_grads(wqa, woa, n3, n1, DQ3, DQ1, O3, O1, g3, g1)
    zero_more(nz)

    def dw_copies(i):
        g, rb = i // 10, i % 10
        rq = pl.ds(pl.multiple_of(rb * 64, 64), 64)
        cq = pl.ds(pl.multiple_of(g * GW, GW), GW)
        ro = pl.ds(pl.multiple_of(i * 96, 32), 96)
        return [pltpu.make_async_copy(wqa.at[g, rq, :], dwqa_hbm.at[rq, cq], sem_w.at[0]),
                pltpu.make_async_copy(wqb.at[g, rq, :], dwqb_hbm.at[rq, cq], sem_w.at[2]),
                pltpu.make_async_copy(woa.at[ro, :], dwoa_hbm.at[ro, :], sem_w.at[1]),
                pltpu.make_async_copy(wob.at[ro, :], dwob_hbm.at[ro, :], sem_w.at[3])]

    def dw_start(i, c):
        for cp in dw_copies(i):
            cp.start()
        return c
    lax.fori_loop(0, 40, dw_start, 0)
    tail = pl.ds(40 * 96, H * DH - 40 * 96)
    pltpu.make_async_copy(woa.at[tail, :], dwoa_hbm.at[tail, :], sem_w.at[1]).start()
    pltpu.make_async_copy(wob.at[tail, :], dwob_hbm.at[tail, :], sem_w.at[3]).start()

    def b_grads(i, c):
        g, cc = i // (WIN // OC), i % (WIN // OC)
        rhs = outer_rhs(tab[DO4, grp(g), :], tab[DO2, grp(g), :], tab[Q4, grp(g), :], tab[Q2, grp(g), :])
        t0 = g * nbt + cc * (OC // DH)
        a = jnp.concatenate([park_load(1, t0, OC // DH), park_load(1, NG * nbt + t0, OC // DH)], axis=0)
        at = a.T
        rows = pl.ds(pl.multiple_of(cc * OC, OC), OC)
        for r in range(G):
            vb[g * G + r, rows, :] = _dot(at, rhs[2 * r], NN).astype(BF16)
            kb[g * G + r, rows, :] = _dot(at, rhs[2 * r + 1], NN).astype(BF16)
        for k in range(OC // WR):
            src = pl.ds(pl.multiple_of(cc * OC + k * WR, WR), WR)
            dst = pl.ds(pl.multiple_of(SK - WIN + cc * OC + k * WR, WR), WR)
            pltpu.make_async_copy(kb.at[grp(g), src, :], dkb_hbm.at[grp(g), dst, :], sem_o.at[0, 0]).start()
            pltpu.make_async_copy(vb.at[grp(g), src, :], dvb_hbm.at[grp(g), dst, :], sem_o.at[1, 0]).start()
        return c
    lax.fori_loop(0, NG * (WIN // OC), b_grads, 0)
    zero_wait(z0, nz)

    win = pl.ds(SK - WIN, WIN)

    def a_grads(g, stage):
        do3, do1 = tab[DO3, grp(g), :], tab[DO1, grp(g), :]
        rhs = outer_rhs(do3, do1, tab[Q3, grp(g), :], tab[Q1, grp(g), :])
        dl = jnp.concatenate([delta(O3, DO3, g), delta(O1, DO1, g)], axis=0)

        def body(cc, c):
            rows = pl.ds(pl.multiple_of(cc * OC, OC), OC)
            dp = _dot(_pair(do3, do1, 0), va[g * G, rows, :], NT)
            for r in range(1, G):
                dp = dp + _dot(_pair(do3, do1, r), va[g * G + r, rows, :], NT)
            p = park_load(0, g * (SK // DH) + cc * (OC // DH), OC // DH)
            ds = (p.astype(F32) * (dp - dl) * SCALE).astype(BF16)
            at = jnp.concatenate([p, ds], axis=0).T
            part = cc // (WIN // OC)
            srow = (cc % (WIN // OC)) * OC
            for r in range(G):
                va[g * G + r, rows, :] = _dot(at, rhs[2 * r], NN).astype(BF16)
                stage[part * G + r, pl.ds(pl.multiple_of(srow, OC), OC), :] = (
                    _dot(at, rhs[2 * r + 1], NN).astype(BF16))
            for k in range(OC // WR):
                dst = pl.ds(pl.multiple_of(cc * OC + k * WR, WR), WR)
                src = pl.ds(pl.multiple_of(srow + k * WR, WR), WR)
                pltpu.make_async_copy(stage.at[grp(part), src, :], dka_hbm.at[grp(g), dst, :],
                                      sem_o.at[0, 1 + g]).start()
                pltpu.make_async_copy(va.at[grp(g), dst, :], dva_hbm.at[grp(g), dst, :],
                                      sem_o.at[1, 1 + g]).start()
            return c
        lax.fori_loop(0, SK // OC, body, 0)

    def dka_wait(g):
        pltpu.make_async_copy(va.at[grp(g)], dka_hbm.at[grp(g)], sem_o.at[0, 1 + g]).wait()

    def dva_wait(g):
        pltpu.make_async_copy(va.at[grp(g)], dva_hbm.at[grp(g)], sem_o.at[1, 1 + g]).wait()

    pltpu.make_async_copy(kb, dkb_hbm.at[:, win, :], sem_o.at[0, 0]).wait()
    a_grads(0, kb)
    pltpu.make_async_copy(vb, dvb_hbm.at[:, win, :], sem_o.at[1, 0]).wait()
    a_grads(1, vb)
    dka_wait(0)
    a_grads(2, kb)
    dka_wait(1)
    a_grads(3, vb)

    out_copy.wait()
    dx_copy.wait()
    for g in range(NG):
        pltpu.make_async_copy(wqa.at[g], dwqa_hbm.at[:, pl.ds(g * GW, GW)], sem_w.at[0]).wait()
        pltpu.make_async_copy(wqb.at[g], dwqb_hbm.at[:, pl.ds(g * GW, GW)], sem_w.at[2]).wait()
    pltpu.make_async_copy(woa, dwoa_hbm, sem_w.at[1]).wait()
    pltpu.make_async_copy(wob, dwob_hbm, sem_w.at[3]).wait()
    for g in range(NG):
        dva_wait(g)
    dka_wait(2)
    dka_wait(3)


@jax.jit
def pallas_interleave_layers__gqa_block_cached__sliding_block_cached__decode_kernel(
    A_x: jax.Array,
    A_k_cache: jax.Array,
    A_v_cache: jax.Array,
    A_wq: jax.Array,
    A_wo: jax.Array,
    B_x: jax.Array,
    B_k_cache: jax.Array,
    B_v_cache: jax.Array,
    B_wq: jax.Array,
    B_wo: jax.Array,
    grad_out: jax.Array,
):
    del B_x
    cache = (H, SK, DH)
    vec = jax.ShapeDtypeStruct((1, D), BF16)
    kv = jax.ShapeDtypeStruct(cache, BF16)
    wq = jax.ShapeDtypeStruct((D, H * DH), BF16)
    wo = jax.ShapeDtypeStruct((H * DH, D), BF16)
    hbm = pl.BlockSpec(memory_space=pl.ANY)
    outs = pl.pallas_call(
        _kernel,
        in_specs=[hbm] * 10,
        out_specs=[hbm] * 10,
        out_shape=[vec, vec, kv, kv, wq, wo, kv, kv, wq, wo],
        scratch_shapes=[
            pltpu.VMEM((H, SK, DH), BF16),
            pltpu.VMEM((H, WIN, DH), BF16),
            pltpu.VMEM((H, WIN, DH), BF16),
            pltpu.VMEM((NSLOT, SK, DH), BF16),
            pltpu.VMEM((NG, D, GW), BF16),
            pltpu.VMEM((H * DH, D), BF16),
            pltpu.VMEM((NG, D, GW), BF16),
            pltpu.VMEM((H * DH, D), BF16),
            pltpu.VMEM((H, DH, DH), BF16),
            pltpu.VMEM((16, H, DH), F32),
            pltpu.VMEM((SK // CH, G, CH), F32),
            pltpu.VMEM((G, ZR, DH), BF16),
            pltpu.VMEM((2, 1, D), BF16),
            pltpu.VMEM((2, 1, D), BF16),
            pltpu.SMEM((1,), jnp.int32),
            pltpu.SemaphoreType.DMA((NSLOT,)),
            pltpu.SemaphoreType.DMA((NSLOT,)),
            pltpu.SemaphoreType.DMA((2, NG)),
            pltpu.SemaphoreType.DMA((4,)),
            pltpu.SemaphoreType.DMA((2,)),
            pltpu.SemaphoreType.DMA((1,)),
            pltpu.SemaphoreType.DMA((2, 1 + NG)),
        ],
        compiler_params=pltpu.CompilerParams(
            vmem_limit_bytes=128 * 1024 * 1024,
            flags={"XLA_TPU_FORCE_LP_LLO_SCHEDULER": True}),
    )(A_x.reshape(1, D), A_k_cache.reshape(cache), A_v_cache.reshape(cache), A_wq, A_wo,
      B_k_cache.reshape(cache), B_v_cache.reshape(cache), B_wq, B_wo, grad_out.reshape(1, D))
    out, dx, dka, dva, dwqa, dwoa, dkb, dvb, dwqb, dwob = outs
    return (out.reshape(A_x.shape), dx.reshape(A_x.shape),
            dka.reshape(A_k_cache.shape), dva.reshape(A_v_cache.shape), dwqa, dwoa,
            dkb.reshape(B_k_cache.shape), dvb.reshape(B_v_cache.shape), dwqb, dwob)
```

```python
import jax
import jax.numpy as jnp
from jax import lax
import jax.experimental.pallas as pl
import jax.experimental.pallas.tpu as pltpu

F32 = jnp.float32
BF16 = jnp.bfloat16

D = 640
H = 32
DH = 128
SK = 8192
WIN = 2048
EPS = 1e-5
SCALE = DH ** -0.5

G = 8
NG = H // G
GW = G * DH
NS = 4
QR = SK // NS
NSTEP = QR // DH
DEPTH = 16
NSLOT = 5
KEEP = 3
CH = 256
NCH = SK // CH
OC = 512
WR = 64
ZR = 64
WQ_ROWS, WQ_COLS = 8, 2048
WO_ROWS = 32
NWQ = D // NS // WQ_ROWS * (H * DH // WQ_COLS)
NWO = H * DH // NS // WO_ROWS
NZ = NG * (SK - WIN) // ZR

NN = (((1,), (0,)), ((), ()))
NT = (((1,), (1,)), ((), ()))
TN = (((0,), (0,)), ((), ()))

Q1, Q2, Q3, O1, O2, O3, Q4, O4, DO1, DO2, DO3, DO4, DQ1, DQ2, DQ3, DQ4 = range(16)
EARLY_TABLES = 6
X, N1, N2, N3, R1, R2, R3, G4, N4, R4, G1, G2, G3 = range(13)
EARLY_VECTORS = 8


def _dot(a, b, dims):
    return lax.dot_general(a, b, dims, preferred_element_type=F32)


def _row_ids():
    return lax.broadcasted_iota(jnp.int32, (G, DH), 0)


def _only_row(x, r):
    return jnp.where(_row_ids() == r, x, 0.0)


def _block_diag(x):
    return jnp.concatenate([_only_row(x, r) for r in range(G)], axis=1)


def _compact(y):
    out = y[:, :DH]
    for r in range(1, G):
        out = jnp.where(_row_ids() == r, y[:, r * DH:(r + 1) * DH], out)
    return out


def _pair(a, b, r):
    return jnp.concatenate([_only_row(a, r), _only_row(b, r)], axis=0).astype(BF16)


def _layernorm(x):
    mean = jnp.mean(x, axis=-1, keepdims=True)
    xc = x - mean
    var = jnp.mean(xc * xc, axis=-1, keepdims=True)
    rstd = 1.0 / jnp.sqrt(var + EPS)
    return xc * rstd, rstd


def _layernorm_bwd(dn, n, rstd):
    return rstd * (dn - jnp.mean(dn, axis=-1, keepdims=True)
                   - n * jnp.mean(dn * n, axis=-1, keepdims=True))


def _softmax(s):
    e = jnp.exp(s - jnp.max(s, axis=-1, keepdims=True))
    return e * (1.0 / jnp.sum(e, axis=-1, keepdims=True))


def _dense_softmax(tiles, span):
    def per_query(op, reduce, parts):
        v = parts[0]
        for part in parts[1:]:
            v = op(v, part)
        v = reduce(v, axis=1, keepdims=True)
        return jnp.concatenate(
            [jnp.broadcast_to(reduce(v[r:r + span], axis=0, keepdims=True), (span, 1))
             for r in range(0, G, span)], axis=0)
    tiles = [t * SCALE for t in tiles]
    top = per_query(jnp.maximum, jnp.max, tiles)
    e = [jnp.exp(t - top) for t in tiles]
    inv = 1.0 / per_query(jnp.add, jnp.sum, e)
    return jnp.concatenate([t * inv for t in e], axis=0)


def _ds(start, size):
    if isinstance(start, int):
        return pl.ds(start, size)
    return pl.ds(pl.multiple_of(start, size), size)


def _loop(lo, hi, body):
    def step(i, carry):
        body(i)
        return carry
    if not (isinstance(lo, int) and isinstance(hi, int)) or hi > lo:
        lax.fori_loop(lo, hi, step, 0)


def _kernel(x_hbm, ka_hbm, va_hbm, wqa_hbm, woa_hbm, kb_hbm, vb_hbm, wqb_hbm, wob_hbm, g_hbm,
            out_hbm, dx_hbm, dka_hbm, dva_hbm, dwqa_hbm, dwoa_hbm, dkb_hbm, dvb_hbm, dwqb_hbm, dwob_hbm,
            va, kvb, ka, wqa, woa, wqb, wob, m1, zeros, tables, vectors,
            sem_read, sem_dw, sem_vec, sem_zero, sem_stage, sem_dv):
    kb, vb = kvb.at[0], kvb.at[1]
    tab = [tables.at[i] for i in range(EARLY_TABLES)]
    vec_at = [(vectors, i) for i in range(EARLY_VECTORS)]

    def grp(g):
        return _ds(g * G, G)

    def step_start(view, n):
        src, dst = view
        sem = sem_read.at[n % DEPTH]
        slow = pl.ds(0, NS - 1)
        pltpu.make_async_copy(src.at[NS - 1], dst.at[NS - 1], sem).start(priority=0)
        pltpu.make_async_copy(src.at[slow], dst.at[slow], sem).start(priority=1)

    def step_wait(view, n):
        pltpu.make_async_copy(*view, sem_read.at[n % DEPTH]).wait()

    def wq_view(src, dst, j):
        per = H * DH // WQ_COLS
        idx = (slice(None), _ds(j // per * WQ_ROWS, WQ_ROWS), _ds(j % per * WQ_COLS, WQ_COLS))
        return src.at[idx], dst.at[idx]

    def wo_view(src, dst, j):
        idx = (slice(None), _ds(j * WO_ROWS, WO_ROWS), slice(None))
        return src.at[idx], dst.at[idx]

    def b_views(j):
        heads, c = _ds(j // (WIN // DH) * NS, NS), j % (WIN // DH)
        return [(src.at[heads, _ds(SK - WIN + c * DH, DH), :], dst.at[heads, _ds(c * DH, DH), :])
                for src, dst in ((kb_hbm, kb), (vb_hbm, vb))]

    def k_view(head, slot, c):
        rows = _ds(c * DH, DH)
        return ka_hbm.at[head, :, rows, :], ka.at[slot, :, rows, :]

    def v_view(head, c):
        rows = _ds(c * DH, DH)
        return va_hbm.at[head, :, rows, :], va.at[head, :, rows, :]

    def slot1(head):
        return (head + NSLOT - H % NSLOT) % NSLOT

    def pair_view(m, j):
        return k_view(m + 1, slot1(m + 1), j // 2) if j % 2 == 0 else v_view(m, j // 2)

    def zero_copy(dst, i, sem=0):
        per = NZ // NG
        return pltpu.make_async_copy(zeros, dst.at[grp(i // per), _ds(i % per * ZR, ZR), :], sem_zero.at[sem])

    def zero_start(lo, hi):
        if isinstance(lo, int):
            _loop(min(lo, NZ), min(hi, NZ), lambda i: zero_copy(dkb_hbm, i).start())
            _loop(max(lo, NZ) - NZ, max(hi, NZ) - NZ, lambda i: zero_copy(dvb_hbm, i).start())
        else:
            _loop(jnp.minimum(lo, NZ), jnp.minimum(hi, NZ), lambda i: zero_copy(dkb_hbm, i).start())
            _loop(jnp.maximum(lo, NZ) - NZ, jnp.maximum(hi, NZ) - NZ, lambda i: zero_copy(dvb_hbm, i).start())

    issued = [0]

    def take_zeros(n):
        issued[0] += n
        assert issued[0] <= 2 * NZ
        return issued[0] - n

    def zero_more(n):
        lo = take_zeros(n)
        zero_start(lo, lo + n)

    def loop_with_zeros(count, n, body):
        lo = take_zeros(count * n)

        def both(i):
            body(i)
            zero_start(lo + i * n, lo + (i + 1) * n)
        _loop(0, count, both)

    def vec(i):
        ref, row = vec_at[i]
        return jnp.broadcast_to(ref[row:row + 1, :], (G, D))

    def put(i, val):
        ref, row = vec_at[i]
        ref[row:row + 1, :] = jnp.broadcast_to(val, (G, D))[0:1, :]

    def weight(w, g):
        return w[g] if w.shape[-1] == D else w[:, :, _ds(g * GW, GW)].reshape(D, GW)

    def to_heads_group(vector, w, dims, dst, g):
        tab[dst][grp(g), :] = _compact(_dot(vector.astype(BF16), weight(w, g), dims))

    def to_heads(vector, w, dims, dst):
        _loop(0, NG, lambda g: to_heads_group(vector, w, dims, dst, g))

    def from_heads(src, w, dims):
        def body(g, acc):
            return acc + _dot(_block_diag(tab[src][grp(g), :]).astype(BF16), weight(w, g), dims)
        acc = lax.fori_loop(0, NG, body, jnp.zeros((G, D), F32))
        return jnp.broadcast_to(jnp.sum(acc, axis=0, keepdims=True), (G, D))

    def normalise(n, r):
        norm, rstd = _layernorm(vec(X))
        put(n, norm)
        put(r, rstd)

    def add_residual(wo, o):
        put(X, vec(X) + from_heads(o, wo, NN))

    def grad_below(wq, dq, g, n, r):
        return vec(g) + _layernorm_bwd(from_heads(dq, wq, NT), vec(n), vec(r))

    def delta(o, do, g):
        return jnp.sum(tab[o][grp(g), :] * tab[do][grp(g), :], axis=1, keepdims=True)

    def head_row(t, head):
        return jnp.broadcast_to(tab[t][pl.ds(head, 1), :], (G, DH))

    def chunk(ref, i, c):
        return ref[i, c // (QR // CH), pl.ds(c % (QR // CH) * CH, CH), :]

    def add_scores(s, q, span, slot, c):
        y = _dot(q, chunk(ka, slot, c), NT)
        for t in range(CH // DH):
            r = (c * (CH // DH) + t) % span
            tile = y[:, t * DH:(t + 1) * DH]
            if r == 0:
                s.append(tile)
            else:
                s[-1] = jnp.where(_row_ids() % span == r, tile, s[-1])

    def first_probs(probs, q, span, slot):
        s = []
        for c in range(NCH):
            add_scores(s, q.astype(BF16), span, slot, c)
        probs[pl.ds(0, len(s) * G), :] = _dense_softmax(s, span)

    def a_head(probs, span, slot, head, q_next, slot_next, dma):
        qb = q_next.astype(BF16)
        acc = jnp.zeros((DH + 16, DH), F32)
        ksum = jnp.zeros((DH, DH), F32)
        s = []
        for c in range(NCH):
            if c % 2 == 0:
                dma(c // 2)
            add_scores(s, qb, span, slot_next, c)
            p = jnp.concatenate(
                [jnp.broadcast_to(probs[pl.ds(t // span * G + t % span, 1), :], (G, DH))
                 for t in range(c * (CH // DH), (c + 1) * (CH // DH))], axis=1)
            kp = chunk(ka, slot, c).T.astype(F32) * jnp.concatenate([p] * (DH // G), axis=0)
            for t in range(CH // DH):
                ksum = ksum + kp[:, t * DH:(t + 1) * DH]
            lhs = jnp.concatenate([kp, p, p], axis=0).astype(BF16)
            acc = acc + _dot(lhs, chunk(va, head, c), NN)
        o = acc[DH:DH + 1, :]
        kbar = jnp.sum(ksum, axis=1, keepdims=True)
        return o, (acc[:DH, :] - kbar * o).astype(BF16), _dense_softmax(s, span)

    def apply_m(m_of_head, src, dst):
        def body(g):
            do = tab[src][grp(g), :]
            dq = jnp.zeros((G, DH), F32)
            for r in range(G):
                dq = dq + _dot(_only_row(do, r).astype(BF16), m_of_head(g * G + r), NT)
            tab[dst][grp(g), :] = dq * SCALE
        _loop(0, NG, body)

    def p_at(head, row0=0, rows=DH):
        return 0, head // NSTEP, _ds(head % NSTEP * DH + row0, rows), slice(None)

    def m3_at(head):
        return 0, NS // 2 + head // NSTEP, _ds(head % NSTEP * DH, DH), slice(None)

    def park_load(slot, tile0, n):
        val = ka[slot, 0, _ds(tile0 * 16, n * 16), :]
        return jnp.concatenate([val[t * 16:(t + 1) * 16, :] for t in range(n)], axis=1)

    def park_store(slot, tile0, val):
        n = val.shape[1] // DH
        ka[slot, 0, _ds(tile0 * 16, n * 16), :] = jnp.concatenate(
            [val[:, t * DH:(t + 1) * DH] for t in range(n)], axis=0)

    def gather_probs(g, slot):
        span, rows = G // 2, 32

        def body(i):
            src = [ka[p_at(g * G + r, i * rows, rows)].astype(F32) for r in range(G)]
            tiles = []
            for t in range(rows // G * span):
                halves = []
                for k in range(2):
                    j = t // span * G + k * span + t % span
                    out = jnp.broadcast_to(src[0][j:j + 1, :], (G, DH))
                    for r in range(1, G):
                        out = jnp.where(_row_ids() == r, jnp.broadcast_to(src[r][j:j + 1, :], (G, DH)), out)
                    halves.append(out)
                tiles.append(jnp.concatenate(halves, axis=0).astype(BF16))
            park_store(slot, i * len(tiles), jnp.concatenate(tiles, axis=1))
        _loop(0, DH // rows, body)

    def b_scores(lhs_of_row, ref, g):
        s = _dot(lhs_of_row(0), ref[g * G], NT)
        for r in range(1, G):
            s = s + _dot(lhs_of_row(r), ref[g * G + r], NT)
        return s

    def b_mix(p, ref, g):
        pb = p.astype(BF16)
        out = _dot(pb, ref[g * G], NN)
        for r in range(1, G):
            out = jnp.where(_row_ids() == r, _dot(pb, ref[g * G + r], NN), out)
        return out

    def outer_rhs(do_a, do_b, q_a, q_b):
        zero = jnp.zeros((16, DH), BF16)
        return [(jnp.concatenate([_pair(do_a, do_b, r), zero], axis=0),
                 jnp.concatenate([zero, _pair(q_a, q_b, r)], axis=0)) for r in range(G)]

    def read_phases(probs, keep, xin):
        x_copy = pltpu.make_async_copy(x_hbm, xin.at[0], sem_vec.at[0])
        g_copy = pltpu.make_async_copy(g_hbm, xin.at[1], sem_vec.at[1])

        segments = [
            (NWQ, lambda j: [wq_view(wqa_hbm, wqa, j), wq_view(wqb_hbm, wqb, j)]),
            (NWO, lambda j: [wo_view(woa_hbm, woa, j), wo_view(wob_hbm, wob, j)]),
            (H // NS * (WIN // DH), b_views),
        ]
        lead_in = [k_view(0, slot1(0), c) for c in range(NSTEP)]
        lead_in += [pair_view(m, j) for m in range(2) for j in range(2 * NSTEP)]
        lag = DEPTH // 2
        for j in range(lag):
            for k, view in enumerate(segments[0][1](j)):
                step_start(view, 2 * j + k)
            if j == 0:
                x_copy.start()
                g_copy.start()
        zeros[...] = jnp.zeros(zeros.shape, BF16)
        for si, (count, views) in enumerate(segments):
            assert count % lag == 0

            def advance(j, ahead, views=views):
                for k, (old, new) in enumerate(zip(views(j), ahead)):
                    step_wait(old, 2 * j + k)
                    step_start(new, 2 * j + k)

            def most(j, si=si, views=views, advance=advance):
                advance(j, views(j + lag))
                if si == 2:
                    pl.when(jnp.logical_and(j % G == G - 1, j < NG * G))(
                        lambda: to_heads_group(vec(N1), wqa, NN, Q1, j // G))
            _loop(0, count - lag, most)
            if si + 1 < len(segments):
                _loop(count - lag, count, lambda j, nxt=segments[si + 1][1], advance=advance, count=count:
                      advance(j, nxt(j + lag - count)))
            else:
                for j in range(count - lag, count):
                    advance(j, lead_in[2 * (j + lag - count):][:2])
            if si == 1:
                x_copy.wait()
                g_copy.wait()
                put(X, xin[0].astype(F32))
                put(G4, xin[1].astype(F32))
                normalise(N1, R1)
        for n in range(3 * NSTEP):
            step_wait(lead_in[n], n)
            step_start(lead_in[n + DEPTH], n)

        first_probs(probs, head_row(Q1, 0), G, slot1(0))
        kept = H - NSLOT - 1
        lead0 = 0
        lead0_at = take_zeros(lead0)
        first = take_zeros(64 - lead0)

        def layer1(h):
            def dma(i):
                if lead0 - NSTEP + i >= 0:
                    pl.when(h == H - 2)(lambda: zero_copy(dkb_hbm, lead0_at + lead0 - NSTEP + i).start())
                for j in (2 * i, 2 * i + 1):
                    pl.when(h + 2 - j % 2 < H)(lambda: step_wait(pair_view(h + 1, j), j))
                    m, k = h + 1 + (j + DEPTH) // (2 * NSTEP), (j + DEPTH) % (2 * NSTEP)
                    pl.when(m + 1 - k % 2 < H)(lambda: step_start(pair_view(m, k), j))

            nxt = jnp.minimum(h + 1, H - 1)
            o, m, p = a_head(probs, G, slot1(h), h, head_row(Q1, nxt), slot1(nxt), dma)
            m1[h] = m
            tab[O1][pl.ds(h, 1), :] = o
            probs[pl.ds(0, SK // DH), :] = p

            @pl.when(h == kept)
            def _():
                keep[...] = ka[slot1(kept), :, pl.ds(0, KEEP * DH), :]
            pl.when(h == H - 2)(lambda: zero_start(first, 64))
        _loop(0, H, layer1)
        zero_more(13)
        add_residual(woa, O1)
        normalise(N2, R2)
        to_heads(vec(N2), wqb, NN, Q2)
        zero_more(18)

        def layer2(g):
            q = tab[Q2][grp(g), :]
            p = _softmax(b_scores(lambda r: _only_row(q, r).astype(BF16), kb, g) * SCALE)
            tab[O2][grp(g), :] = b_mix(p, vb, g)
        loop_with_zeros(NG, 15, layer2)
        add_residual(wob, O2)
        normalise(N3, R3)
        to_heads(vec(N3), wqa, NN, Q3)
        zero_more(4)
        between_reads = issued[0]
        last = take_zeros(1)
        zero_copy(dkb_hbm, last, 1).start()

        ring = NSLOT - 1
        lead = 16
        lead_at = take_zeros(lead)
        burst = 56
        first = take_zeros(burst)
        assert first <= NZ

        def head3(i):
            return (i + H - NSLOT) % H

        def slot3(i):
            return jnp.where(i == 0, 0, 1 + (i + ring - 1) % ring)

        def queries(head):
            return jnp.where(_row_ids() < G // 2, head_row(Q3, head), head_row(Q1, head))

        first_probs(probs, queries(head3(0)), G // 2, 0)

        def layer3(i):
            def streamed(a, c):
                return jnp.logical_and(a >= NSLOT, a < (H - 1 if c < KEEP else H))

            def dma(c):
                for back in range(2):
                    k = lead - (back + 1) * NSTEP + c
                    if k >= 0:
                        pl.when(i == H - 3 - back)(lambda: zero_copy(dkb_hbm, lead_at + k, 1).start())
                pl.when(streamed(i + 2, c))(lambda: step_wait(k_view(head3(i + 2), slot3(i + 2), c), c))
                pl.when(streamed(i + 3, c))(lambda: step_start(k_view(head3(i + 3), slot3(i + 3), c), c))

            @pl.when(i == NSLOT - 3)
            def _():
                _loop(0, between_reads, lambda k: zero_copy(dkb_hbm, k).wait())

            head, nxt = head3(i), jnp.minimum(i + 1, H - 1)
            o, m, p = a_head(probs, G // 2, slot3(i), head, queries(head3(nxt)), slot3(nxt), dma)
            ka[m3_at(head)] = m
            tab[O3][pl.ds(head, 1), :] = o
            ka[p_at(head)] = probs[...].astype(BF16)
            probs[...] = p

            @pl.when(i == H - 3)
            def _():
                zero_start(first, first + burst)
                ka[1 + (H + ring - 2) % ring, :, pl.ds(0, KEEP * DH), :] = keep[...]
        assert DEPTH == NSTEP
        _loop(0, H, layer3)
        _loop(last, first, lambda k: zero_copy(dkb_hbm, k, 1).wait())
        waited.append(first)

    def gradient_phases(late_tables, late_vectors, xout):
        tab.extend(late_tables.at[i] for i in range(late_tables.shape[0]))
        vec_at.extend((late_vectors, i) for i in range(late_vectors.shape[0]))
        zero_more(30)
        add_residual(woa, O3)
        normalise(N4, R4)
        to_heads(vec(N4), wqb, NN, Q4)
        zero_more(18)
        to_heads(vec(G4), wob, NT, DO4)
        zero_more(12)

        nbt = WIN // DH

        def layer4(g):
            q4, q2 = tab[Q4][grp(g), :], tab[Q2][grp(g), :]
            p = _softmax(b_scores(lambda r: _pair(q4, q2, r), kb, g) * SCALE)
            park_store(1, g * nbt, p.astype(BF16))
            p4 = p[:G, :]
            tab[O4][grp(g), :] = b_mix(p4, vb, g)
            do = tab[DO4][grp(g), :]
            dp = b_scores(lambda r: _only_row(do, r).astype(BF16), vb, g)
            ds = p4 * (dp - delta(O4, DO4, g)) * SCALE
            park_store(1, (NG + g) * nbt, jnp.concatenate([ds, ds], axis=0).astype(BF16))
            tab[DQ4][grp(g), :] = b_mix(ds, kb, g)
        loop_with_zeros(NG, 29, layer4)
        add_residual(wob, O4)
        xout[0] = vec(X)[0:1, :].astype(BF16)
        out_copy = pltpu.make_async_copy(xout.at[0], out_hbm, sem_vec.at[0])
        out_copy.start()
        put(G3, grad_below(wqb, DQ4, G4, N4, R4))
        zero_more(22)

        to_heads(vec(G3), woa, NT, DO3)
        apply_m(lambda h: ka[m3_at(h)], DO3, DQ3)
        zero_more(18)
        put(G2, grad_below(wqa, DQ3, G3, N3, R3))
        zero_more(14)

        to_heads(vec(G2), wob, NT, DO2)
        zero_more(12)

        def layer2_bwd(g):
            do = tab[DO2][grp(g), :]
            dp = b_scores(lambda r: _only_row(do, r).astype(BF16), vb, g)
            p2 = park_load(1, g * nbt, nbt).astype(F32)[G:, :]
            ds = p2 * (dp - delta(O2, DO2, g)) * SCALE
            ds4 = park_load(1, (NG + g) * nbt, nbt).astype(F32)[:G, :]
            park_store(1, (NG + g) * nbt, jnp.concatenate([ds4, ds], axis=0).astype(BF16))
            tab[DQ2][grp(g), :] = b_mix(ds, kb, g)
        loop_with_zeros(NG, 14, layer2_bwd)
        put(G1, grad_below(wqb, DQ2, G2, N2, R2))
        zero_more(14)

        to_heads(vec(G1), woa, NT, DO1)
        apply_m(lambda h: m1[h], DO1, DQ1)
        zero_more(18)
        xout[1] = grad_below(wqa, DQ1, G1, N1, R1)[0:1, :].astype(BF16)
        dx_copy = pltpu.make_async_copy(xout.at[1], dx_hbm, sem_vec.at[1])
        dx_copy.start()
        zero_more(24)

        def b_grads(i):
            g, c = i // (WIN // OC), i % (WIN // OC)
            rhs = outer_rhs(tab[DO4][grp(g), :], tab[DO2][grp(g), :], tab[Q4][grp(g), :], tab[Q2][grp(g), :])
            t0 = g * nbt + c * (OC // DH)
            at = jnp.concatenate([park_load(1, t0, OC // DH), park_load(1, NG * nbt + t0, OC // DH)], axis=0).T
            for r in range(G):
                vb[g * G + r, _ds(c * OC, OC), :] = _dot(at, rhs[r][0], NN).astype(BF16)
                kb[g * G + r, _ds(c * OC, OC), :] = _dot(at, rhs[r][1], NN).astype(BF16)
        loop_with_zeros(NG * WIN // OC, 9, b_grads)
        zero_more(2 * NZ - issued[0])

        def weight_grads(wq, wo, na, nb, dqa, dqb, oa, ob, ga, gb, which):
            unroll = 4
            per = NG * WIN // WR // (H // unroll)

            def db_start(k):
                g, row = k // (WIN // WR), k % (WIN // WR) * WR
                pltpu.make_async_copy(kvb.at[which, grp(g), _ds(row, WR), :],
                                      (dkb_hbm, dvb_hbm)[which].at[grp(g), _ds(SK - WIN + row, WR), :],
                                      sem_stage.at[which]).start()

            def body(i):
                _loop(i * per, (i + 1) * per, db_start)
                g, r0 = i // (G // unroll), i % (G // unroll) * unroll
                ns = jnp.concatenate([vec(na), vec(nb)], axis=0).astype(BF16).T
                gs = jnp.concatenate([vec(ga), vec(gb)], axis=0).astype(BF16)
                for k in range(unroll):
                    r = r0 + k
                    dq = _pair(tab[dqa][grp(g), :], tab[dqb][grp(g), :], r)
                    wq[:, :, _ds(g * GW + r * DH, DH)] = _dot(ns, dq, NN).astype(BF16).reshape(NS, D // NS, DH)
                    o = _pair(tab[oa][grp(g), :], tab[ob][grp(g), :], r)
                    wo[g, _ds(r * DH, DH), :] = _dot(o, gs, TN).astype(BF16)
            _loop(0, H // unroll, body)

        weight_grads(wqb, wob, N4, N2, DQ4, DQ2, O4, O2, G4, G2, 0)
        weight_grads(wqa, woa, N3, N1, DQ3, DQ1, O3, O1, G3, G1, 1)
        dw = ((wqa, dwqa_hbm), (wqb, dwqb_hbm), (woa, dwoa_hbm), (wob, dwob_hbm))

        def dw_start(view, first, j):
            for k in (first, first + 1):
                pltpu.make_async_copy(*view(*dw[k], j), sem_dw.at[k]).start()

        def staged_wait(k):
            stage = kvb.at[k % 2]
            pltpu.make_async_copy(stage, stage, sem_stage.at[k]).wait()

        def a_rows(i):
            return i // (QR // WR), _ds(i % (QR // WR) * WR, WR)

        def dv_start(g, i):
            idx = (grp(g),) + a_rows(i)
            pltpu.make_async_copy(va.at[idx], dva_hbm.at[idx], sem_dv.at[0]).start()

        def dk_start(g, i):
            part, rows = a_rows(i)
            pltpu.make_async_copy(kvb.at[g % 2, grp(part), rows], dka_hbm.at[grp(g), part, rows],
                                  sem_stage.at[2 + g]).start()

        def a_grads(g):
            staged_wait(g)
            gather_probs(g, 2)
            do3, do1 = tab[DO3][grp(g), :], tab[DO1][grp(g), :]
            rhs = outer_rhs(do3, do1, tab[Q3][grp(g), :], tab[Q1][grp(g), :])
            dl = jnp.concatenate([delta(O3, DO3, g), delta(O1, DO1, g)], axis=0)
            half = SK // OC // 2
            per = SK // WR // half

            def body(c):
                part, rows = c // (QR // OC), _ds(c % (QR // OC) * OC, OC)
                dp = _dot(_pair(do3, do1, 0), va[g * G, part, rows, :], NT)
                for r in range(1, G):
                    dp = dp + _dot(_pair(do3, do1, r), va[g * G + r, part, rows, :], NT)
                p = park_load(2, c * (OC // DH), OC // DH)
                ds = (p.astype(F32) * (dp - dl) * SCALE).astype(BF16)
                at = jnp.concatenate([p, ds], axis=0).T
                for r in range(G):
                    va[g * G + r, part, rows, :] = _dot(at, rhs[r][0], NN).astype(BF16)
                    kvb[g % 2, part * G + r, rows, :] = _dot(at, rhs[r][1], NN).astype(BF16)

                @pl.when(c >= half)
                def _():
                    _loop((c - half) * per, (c - half + 1) * per, lambda i: dv_start(g, i))

                @pl.when(jnp.logical_and(c < half, g > 0))
                def _():
                    _loop(c * per, (c + 1) * per, lambda i: dk_start(g - 1, i))

                @pl.when(jnp.logical_and(c < half // 2, g == 0))
                def _():
                    n = NWO // (half // 2)
                    _loop(c * n, (c + 1) * n, lambda j: dw_start(wo_view, 2, j))

                @pl.when(jnp.logical_and(c // (half // 2) == 1, g == 0))
                def _():
                    n = NWQ // (half // 2)
                    _loop((c - half // 2) * n, (c - half // 2 + 1) * n, lambda j: dw_start(wq_view, 0, j))
            _loop(0, SK // OC, body)
        _loop(0, NG, a_grads)
        _loop(0, SK // WR, lambda i: dk_start(NG - 1, i))

        _loop(waited[0], NZ, lambda i: zero_copy(dkb_hbm, i).wait())
        _loop(0, NZ, lambda i: zero_copy(dvb_hbm, i).wait())
        out_copy.wait()
        dx_copy.wait()
        for k, pair in enumerate(dw):
            pltpu.make_async_copy(*pair, sem_dw.at[k]).wait()
        pltpu.make_async_copy(va, dva_hbm, sem_dv.at[0]).wait()
        staged_wait(NG)
        staged_wait(NG + 1)

    waited = []
    pl.run_scoped(read_phases,
                  pltpu.VMEM((2 * SK // DH, DH), F32),
                  pltpu.VMEM((NS, KEEP * DH, DH), BF16),
                  pltpu.VMEM((2, 1, D), BF16))
    pl.run_scoped(gradient_phases,
                  pltpu.VMEM((16 - EARLY_TABLES, H, DH), F32),
                  pltpu.VMEM((13 - EARLY_VECTORS, D), F32),
                  pltpu.VMEM((2, 1, D), BF16))


@jax.jit
def pallas_interleave_layers__gqa_block_cached__sliding_block_cached__decode_kernel(
    A_x: jax.Array,
    A_k_cache: jax.Array,
    A_v_cache: jax.Array,
    A_wq: jax.Array,
    A_wo: jax.Array,
    B_x: jax.Array,
    B_k_cache: jax.Array,
    B_v_cache: jax.Array,
    B_wq: jax.Array,
    B_wo: jax.Array,
    grad_out: jax.Array,
):
    del B_x
    a_view = (H, NS, QR, DH)
    b_view = (H, SK, DH)
    wq_view = (NS, D // NS, H * DH)
    wo_view = (NG, GW, D)
    vec, a_out, b_out, wq, wo = (
        jax.ShapeDtypeStruct(s, BF16) for s in ((1, D), a_view, b_view, wq_view, wo_view))
    hbm = pl.BlockSpec(memory_space=pl.ANY)
    out, dx, dka, dva, dwqa, dwoa, dkb, dvb, dwqb, dwob = pl.pallas_call(
        _kernel,
        in_specs=[hbm] * 10,
        out_specs=[hbm] * 10,
        out_shape=[vec, vec, a_out, a_out, wq, wo, b_out, b_out, wq, wo],
        scratch_shapes=[
            pltpu.VMEM(a_view, BF16),
            pltpu.VMEM((2, H, WIN, DH), BF16),
            pltpu.VMEM((NSLOT, NS, QR, DH), BF16),
            pltpu.VMEM(wq_view, BF16),
            pltpu.VMEM(wo_view, BF16),
            pltpu.VMEM(wq_view, BF16),
            pltpu.VMEM(wo_view, BF16),
            pltpu.VMEM((H, DH, DH), BF16),
            pltpu.VMEM((G, ZR, DH), BF16),
            pltpu.VMEM((EARLY_TABLES, H, DH), F32),
            pltpu.VMEM((EARLY_VECTORS, D), F32),
            pltpu.SemaphoreType.DMA((DEPTH,)),
            pltpu.SemaphoreType.DMA((4,)),
            pltpu.SemaphoreType.DMA((2,)),
            pltpu.SemaphoreType.DMA((2,)),
            pltpu.SemaphoreType.DMA((2 + NG,)),
            pltpu.SemaphoreType.DMA((1,)),
        ],
        compiler_params=pltpu.CompilerParams(
            vmem_limit_bytes=128 * 1024 * 1024,
            disable_bounds_checks=True,
            flags={"XLA_TPU_FORCE_LP_LLO_SCHEDULER": True, "XLA_TPU_RESCHEDULE_DMA_DONES": True}),
    )(A_x.reshape(1, D), A_k_cache.reshape(a_view), A_v_cache.reshape(a_view),
      A_wq.reshape(wq_view), A_wo.reshape(wo_view),
      B_k_cache.reshape(b_view), B_v_cache.reshape(b_view),
      B_wq.reshape(wq_view), B_wo.reshape(wo_view), grad_out.reshape(1, D))
    return (out.reshape(A_x.shape), dx.reshape(A_x.shape),
            dka.reshape(A_k_cache.shape), dva.reshape(A_v_cache.shape),
            dwqa.reshape(A_wq.shape), dwoa.reshape(A_wo.shape),
            dkb.reshape(B_k_cache.shape), dvb.reshape(B_v_cache.shape),
            dwqb.reshape(B_wq.shape), dwob.reshape(B_wo.shape))
```

```python
import jax
import jax.numpy as jnp
from jax import lax
import jax.experimental.pallas as pl
import jax.experimental.pallas.tpu as pltpu

F32 = jnp.float32
BF16 = jnp.bfloat16

D = 640
H = 32
DH = 128
SK = 8192
WIN = 2048
EPS = 1e-5
SCALE = DH ** -0.5

G = 8
NG = H // G
GW = G * DH
NS = 4
QR = SK // NS
NSTEP = QR // DH
DEPTH = 16
NSLOT = 5
KEEP = 3
CH = 256
NCH = SK // CH
OC = 512
WR = 64
ZR = 64
WQ_ROWS, WQ_COLS = 8, 2048
WO_ROWS = 32
NWQ = D // NS // WQ_ROWS * (H * DH // WQ_COLS)
NWO = H * DH // NS // WO_ROWS
NZ = NG * (SK - WIN) // ZR

NN = (((1,), (0,)), ((), ()))
NT = (((1,), (1,)), ((), ()))
TN = (((0,), (0,)), ((), ()))

Q1, Q2, Q3, O1, O2, O3, Q4, O4, DO1, DO2, DO3, DO4, DQ1, DQ2, DQ3, DQ4 = range(16)
EARLY_TABLES = 6
X, N1, N2, N3, R1, R2, R3, G4, N4, R4, G1, G2, G3 = range(13)
EARLY_VECTORS = 8


def _dot(a, b, dims):
    return lax.dot_general(a, b, dims, preferred_element_type=F32)


def _row_ids():
    return lax.broadcasted_iota(jnp.int32, (G, DH), 0)


def _only_row(x, r):
    return jnp.where(_row_ids() == r, x, 0.0)


def _block_diag(x):
    return jnp.concatenate([_only_row(x, r) for r in range(G)], axis=1)


def _compact(y):
    out = y[:, :DH]
    for r in range(1, G):
        out = jnp.where(_row_ids() == r, y[:, r * DH:(r + 1) * DH], out)
    return out


def _pair(a, b, r):
    return jnp.concatenate([_only_row(a, r), _only_row(b, r)], axis=0).astype(BF16)


def _layernorm(x):
    mean = jnp.mean(x, axis=-1, keepdims=True)
    xc = x - mean
    var = jnp.mean(xc * xc, axis=-1, keepdims=True)
    rstd = 1.0 / jnp.sqrt(var + EPS)
    return xc * rstd, rstd


def _layernorm_bwd(dn, n, rstd):
    return rstd * (dn - jnp.mean(dn, axis=-1, keepdims=True)
                   - n * jnp.mean(dn * n, axis=-1, keepdims=True))


def _softmax(s):
    e = jnp.exp(s - jnp.max(s, axis=-1, keepdims=True))
    return e * (1.0 / jnp.sum(e, axis=-1, keepdims=True))


def _dense_softmax(tiles, span):
    def per_query(op, reduce, parts):
        v = parts[0]
        for part in parts[1:]:
            v = op(v, part)
        v = reduce(v, axis=1, keepdims=True)
        return jnp.concatenate(
            [jnp.broadcast_to(reduce(v[r:r + span], axis=0, keepdims=True), (span, 1))
             for r in range(0, G, span)], axis=0)
    tiles = [t * SCALE for t in tiles]
    top = per_query(jnp.maximum, jnp.max, tiles)
    e = [jnp.exp(t - top) for t in tiles]
    inv = 1.0 / per_query(jnp.add, jnp.sum, e)
    return jnp.concatenate([t * inv for t in e], axis=0)


def _ds(start, size):
    if isinstance(start, int):
        return pl.ds(start, size)
    return pl.ds(pl.multiple_of(start, size), size)


def _loop(lo, hi, body):
    def step(i, carry):
        body(i)
        return carry
    if not (isinstance(lo, int) and isinstance(hi, int)) or hi > lo:
        lax.fori_loop(lo, hi, step, 0)


def _kernel(x_hbm, ka_hbm, va_hbm, wqa_hbm, woa_hbm, kb_hbm, vb_hbm, wqb_hbm, wob_hbm, g_hbm,
            out_hbm, dx_hbm, dka_hbm, dva_hbm, dwqa_hbm, dwoa_hbm, dkb_hbm, dvb_hbm, dwqb_hbm, dwob_hbm,
            va, kvb, ka, wqa, woa, wqb, wob, m1, zeros, tables, vectors,
            sem_read, sem_dw, sem_vec, sem_zero, sem_stage, sem_dv):
    kb, vb = kvb.at[0], kvb.at[1]
    tab = [tables.at[i] for i in range(EARLY_TABLES)]
    vec_at = [(vectors, i) for i in range(EARLY_VECTORS)]

    def grp(g):
        return _ds(g * G, G)

    def step_start(view, n, urgent=True):
        src, dst = view
        sem = sem_read.at[n % DEPTH]
        slow = pl.ds(0, NS - 1)
        pltpu.make_async_copy(src.at[NS - 1], dst.at[NS - 1], sem).start(priority=0 if urgent else 1)
        pltpu.make_async_copy(src.at[slow], dst.at[slow], sem).start(priority=1)

    def step_wait(view, n):
        pltpu.make_async_copy(*view, sem_read.at[n % DEPTH]).wait()

    def wq_view(src, dst, j):
        per = H * DH // WQ_COLS
        idx = (slice(None), _ds(j // per * WQ_ROWS, WQ_ROWS), _ds(j % per * WQ_COLS, WQ_COLS))
        return src.at[idx], dst.at[idx]

    def wo_view(src, dst, j):
        idx = (slice(None), _ds(j * WO_ROWS, WO_ROWS), slice(None))
        return src.at[idx], dst.at[idx]

    def b_views(j):
        heads, c = _ds(j // (WIN // DH) * NS, NS), j % (WIN // DH)
        return [(src.at[heads, _ds(SK - WIN + c * DH, DH), :], dst.at[heads, _ds(c * DH, DH), :])
                for src, dst in ((kb_hbm, kb), (vb_hbm, vb))]

    def k_view(head, slot, c):
        rows = _ds(c * DH, DH)
        return ka_hbm.at[head, :, rows, :], ka.at[slot, :, rows, :]

    def v_view(head, c):
        rows = _ds(c * DH, DH)
        return va_hbm.at[head, :, rows, :], va.at[head, :, rows, :]

    def slot1(head):
        return (head + NSLOT - H % NSLOT) % NSLOT

    def pair_view(m, j):
        return k_view(m + 1, slot1(m + 1), j // 2) if j % 2 == 0 else v_view(m, j // 2)

    def zero_copy(dst, i, sem=0):
        per = NZ // NG
        return pltpu.make_async_copy(zeros, dst.at[grp(i // per), _ds(i % per * ZR, ZR), :], sem_zero.at[sem])

    def zero_start(lo, hi):
        if isinstance(lo, int):
            _loop(min(lo, NZ), min(hi, NZ), lambda i: zero_copy(dkb_hbm, i).start())
            _loop(max(lo, NZ) - NZ, max(hi, NZ) - NZ, lambda i: zero_copy(dvb_hbm, i).start())
        else:
            _loop(jnp.minimum(lo, NZ), jnp.minimum(hi, NZ), lambda i: zero_copy(dkb_hbm, i).start())
            _loop(jnp.maximum(lo, NZ) - NZ, jnp.maximum(hi, NZ) - NZ, lambda i: zero_copy(dvb_hbm, i).start())

    fill = {"issued": 0, "waited": 0}

    def take_zeros(n):
        fill["issued"] += n
        assert fill["issued"] <= 2 * NZ
        return fill["issued"] - n

    def zero_more(n):
        lo = take_zeros(n)
        zero_start(lo, lo + n)

    def loop_with_zeros(count, n, body):
        lo = take_zeros(count * n)

        def both(i):
            body(i)
            zero_start(lo + i * n, lo + (i + 1) * n)
        _loop(0, count, both)

    def vec(i):
        ref, row = vec_at[i]
        return jnp.broadcast_to(ref[row:row + 1, :], (G, D))

    def put(i, val):
        ref, row = vec_at[i]
        ref[row:row + 1, :] = jnp.broadcast_to(val, (G, D))[0:1, :]

    def weight(w, g):
        return w[g] if w.shape[-1] == D else w[:, :, _ds(g * GW, GW)].reshape(D, GW)

    def to_heads_group(vector, w, dims, dst, g):
        tab[dst][grp(g), :] = _compact(_dot(vector.astype(BF16), weight(w, g), dims))

    def to_heads(vector, w, dims, dst):
        _loop(0, NG, lambda g: to_heads_group(vector, w, dims, dst, g))

    def from_heads(src, w, dims):
        def body(g, acc):
            return acc + _dot(_block_diag(tab[src][grp(g), :]).astype(BF16), weight(w, g), dims)
        acc = lax.fori_loop(0, NG, body, jnp.zeros((G, D), F32))
        return jnp.broadcast_to(jnp.sum(acc, axis=0, keepdims=True), (G, D))

    def normalise(n, r):
        norm, rstd = _layernorm(vec(X))
        put(n, norm)
        put(r, rstd)

    def add_residual(wo, o):
        put(X, vec(X) + from_heads(o, wo, NN))

    def grad_below(wq, dq, g, n, r):
        return vec(g) + _layernorm_bwd(from_heads(dq, wq, NT), vec(n), vec(r))

    def delta(o, do, g):
        return jnp.sum(tab[o][grp(g), :] * tab[do][grp(g), :], axis=1, keepdims=True)

    def head_row(t, head):
        return jnp.broadcast_to(tab[t][pl.ds(head, 1), :], (G, DH))

    def chunk(ref, i, c):
        return ref[i, c // (QR // CH), pl.ds(c % (QR // CH) * CH, CH), :]

    def add_scores(s, q, span, slot, c):
        y = _dot(q, chunk(ka, slot, c), NT)
        for t in range(CH // DH):
            r = (c * (CH // DH) + t) % span
            tile = y[:, t * DH:(t + 1) * DH]
            if r == 0:
                s.append(tile)
            else:
                s[-1] = jnp.where(_row_ids() % span == r, tile, s[-1])

    def first_probs(probs, q, span, slot):
        s = []
        for c in range(NCH):
            add_scores(s, q.astype(BF16), span, slot, c)
        probs[pl.ds(0, len(s) * G), :] = _dense_softmax(s, span)

    def a_head(probs, span, slot, head, q_next, slot_next, dma):
        qb = q_next.astype(BF16)
        acc = jnp.zeros((DH + 16, DH), F32)
        ksum = jnp.zeros((DH, DH), F32)
        s = []
        for c in range(NCH):
            if c % 2 == 0:
                dma(c // 2)
            add_scores(s, qb, span, slot_next, c)
            p = jnp.concatenate(
                [jnp.broadcast_to(probs[pl.ds(t // span * G + t % span, 1), :], (G, DH))
                 for t in range(c * (CH // DH), (c + 1) * (CH // DH))], axis=1)
            kp = chunk(ka, slot, c).T.astype(F32) * jnp.concatenate([p] * (DH // G), axis=0)
            for t in range(CH // DH):
                ksum = ksum + kp[:, t * DH:(t + 1) * DH]
            lhs = jnp.concatenate([kp, p, p], axis=0).astype(BF16)
            acc = acc + _dot(lhs, chunk(va, head, c), NN)
        o = acc[DH:DH + 1, :]
        kbar = jnp.sum(ksum, axis=1, keepdims=True)
        return o, (acc[:DH, :] - kbar * o).astype(BF16), _dense_softmax(s, span)

    def apply_m(m_of_head, src, dst):
        def body(g):
            do = tab[src][grp(g), :]
            dq = jnp.zeros((G, DH), F32)
            for r in range(G):
                dq = dq + _dot(_only_row(do, r).astype(BF16), m_of_head(g * G + r), NT)
            tab[dst][grp(g), :] = dq * SCALE
        _loop(0, NG, body)

    def p_at(head, row0=0, rows=DH):
        return 0, head // NSTEP, _ds(head % NSTEP * DH + row0, rows), slice(None)

    def m3_at(head):
        return 0, NS // 2 + head // NSTEP, _ds(head % NSTEP * DH, DH), slice(None)

    def park_load(slot, tile0, n):
        val = ka[slot, 0, _ds(tile0 * 16, n * 16), :]
        return jnp.concatenate([val[t * 16:(t + 1) * 16, :] for t in range(n)], axis=1)

    def park_store(slot, tile0, val):
        n = val.shape[1] // DH
        ka[slot, 0, _ds(tile0 * 16, n * 16), :] = jnp.concatenate(
            [val[:, t * DH:(t + 1) * DH] for t in range(n)], axis=0)

    def gather_probs(g, slot):
        span, rows = G // 2, 32

        def body(i):
            src = [ka[p_at(g * G + r, i * rows, rows)].astype(F32) for r in range(G)]
            tiles = []
            for t in range(rows // G * span):
                halves = []
                for k in range(2):
                    j = t // span * G + k * span + t % span
                    out = jnp.broadcast_to(src[0][j:j + 1, :], (G, DH))
                    for r in range(1, G):
                        out = jnp.where(_row_ids() == r, jnp.broadcast_to(src[r][j:j + 1, :], (G, DH)), out)
                    halves.append(out)
                tiles.append(jnp.concatenate(halves, axis=0).astype(BF16))
            park_store(slot, i * len(tiles), jnp.concatenate(tiles, axis=1))
        _loop(0, DH // rows, body)

    def b_scores(lhs_of_row, ref, g):
        s = _dot(lhs_of_row(0), ref[g * G], NT)
        for r in range(1, G):
            s = s + _dot(lhs_of_row(r), ref[g * G + r], NT)
        return s

    def b_mix(p, ref, g):
        pb = p.astype(BF16)
        out = _dot(pb, ref[g * G], NN)
        for r in range(1, G):
            out = jnp.where(_row_ids() == r, _dot(pb, ref[g * G + r], NN), out)
        return out

    def outer_rhs(do_a, do_b, q_a, q_b):
        zero = jnp.zeros((16, DH), BF16)
        return [(jnp.concatenate([_pair(do_a, do_b, r), zero], axis=0),
                 jnp.concatenate([zero, _pair(q_a, q_b, r)], axis=0)) for r in range(G)]

    def read_phases(probs, keep, xin):
        x_copy = pltpu.make_async_copy(x_hbm, xin.at[0], sem_vec.at[0])
        g_copy = pltpu.make_async_copy(g_hbm, xin.at[1], sem_vec.at[1])

        segments = [
            (NWQ, lambda j: [wq_view(wqa_hbm, wqa, j), wq_view(wqb_hbm, wqb, j)]),
            (NWO, lambda j: [wo_view(woa_hbm, woa, j), wo_view(wob_hbm, wob, j)]),
            (H // NS * (WIN // DH), b_views),
        ]
        lead_in = [k_view(0, slot1(0), c) for c in range(NSTEP)]
        lead_in += [pair_view(m, j) for m in range(2) for j in range(2 * NSTEP)]
        lag = DEPTH // 2
        for j in range(lag):
            for k, view in enumerate(segments[0][1](j)):
                step_start(view, 2 * j + k, urgent=False)
            if j == 0:
                x_copy.start()
                g_copy.start()
        zeros[...] = jnp.zeros(zeros.shape, BF16)
        for si, (count, views) in enumerate(segments):
            assert count % lag == 0

            def advance(j, ahead, views=views):
                for k, (old, new) in enumerate(zip(views(j), ahead)):
                    step_wait(old, 2 * j + k)
                    step_start(new, 2 * j + k)

            def most(j, si=si, views=views, advance=advance):
                advance(j, views(j + lag))
                if si == 2:
                    pl.when(jnp.logical_and(j % G == G - 1, j < NG * G))(
                        lambda: to_heads_group(vec(N1), wqa, NN, Q1, j // G))
            _loop(0, count - lag, most)
            if si + 1 < len(segments):
                _loop(count - lag, count, lambda j, nxt=segments[si + 1][1], advance=advance, count=count:
                      advance(j, nxt(j + lag - count)))
            else:
                for j in range(count - lag, count):
                    advance(j, lead_in[2 * (j + lag - count):][:2])
            if si == 1:
                x_copy.wait()
                g_copy.wait()
                put(X, xin[0].astype(F32))
                put(G4, xin[1].astype(F32))
                normalise(N1, R1)
        for n in range(3 * NSTEP):
            step_wait(lead_in[n], n)
            step_start(lead_in[n + DEPTH], n)

        first_probs(probs, head_row(Q1, 0), G, slot1(0))
        kept = H - NSLOT - 1
        first = take_zeros(64)

        def layer1(h):
            def dma(i):
                for j in (2 * i, 2 * i + 1):
                    pl.when(h + 2 < H)(lambda: step_wait(pair_view(h + 1, j), j))
                    m, k = h + 1 + (j + DEPTH) // (2 * NSTEP), (j + DEPTH) % (2 * NSTEP)
                    pl.when(m + 1 - k % 2 < H)(lambda: step_start(pair_view(m, k), j))

            nxt = jnp.minimum(h + 1, H - 1)
            o, m, p = a_head(probs, G, slot1(h), h, head_row(Q1, nxt), slot1(nxt), dma)
            m1[h] = m
            tab[O1][pl.ds(h, 1), :] = o
            probs[pl.ds(0, SK // DH), :] = p

            @pl.when(h == kept)
            def _():
                keep[...] = ka[slot1(kept), :, pl.ds(0, KEEP * DH), :]

            @pl.when(h == H - 2)
            def _():
                zero_start(first, first + 64)
                for j in range(1, 2 * NSTEP, 2):
                    step_wait(pair_view(H - 1, j), j)
        _loop(0, H, layer1)
        zero_more(13)
        add_residual(woa, O1)
        normalise(N2, R2)
        to_heads(vec(N2), wqb, NN, Q2)
        zero_more(18)

        def layer2(g):
            q = tab[Q2][grp(g), :]
            p = _softmax(b_scores(lambda r: _only_row(q, r).astype(BF16), kb, g) * SCALE)
            tab[O2][grp(g), :] = b_mix(p, vb, g)
        loop_with_zeros(NG, 15, layer2)
        add_residual(wob, O2)
        normalise(N3, R3)
        to_heads(vec(N3), wqa, NN, Q3)
        zero_more(4)
        between_reads = fill["issued"]
        last = take_zeros(1)
        zero_copy(dkb_hbm, last, 1).start()

        ring = NSLOT - 1
        lead = take_zeros(NSTEP)
        first = take_zeros(56)
        assert first <= NZ

        def head3(i):
            return (i + H - NSLOT) % H

        def slot3(i):
            return jnp.where(i == 0, 0, 1 + (i + ring - 1) % ring)

        def queries(head):
            return jnp.where(_row_ids() < G // 2, head_row(Q3, head), head_row(Q1, head))

        first_probs(probs, queries(head3(0)), G // 2, 0)

        def layer3(i):
            def streamed(a, c):
                return jnp.logical_and(a >= NSLOT, a < (H - 1 if c < KEEP else H))

            def dma(c):
                pl.when(i == H - 3)(lambda: zero_copy(dkb_hbm, lead + c, 1).start())
                pl.when(streamed(i + 2, c))(lambda: step_wait(k_view(head3(i + 2), slot3(i + 2), c), c))
                pl.when(streamed(i + 3, c))(lambda: step_start(k_view(head3(i + 3), slot3(i + 3), c), c))

            @pl.when(i == NSLOT - 3)
            def _():
                _loop(0, between_reads, lambda k: zero_copy(dkb_hbm, k).wait())

            head, nxt = head3(i), jnp.minimum(i + 1, H - 1)
            o, m, p = a_head(probs, G // 2, slot3(i), head, queries(head3(nxt)), slot3(nxt), dma)
            ka[m3_at(head)] = m
            tab[O3][pl.ds(head, 1), :] = o
            ka[p_at(head)] = probs[...].astype(BF16)
            probs[...] = p

            @pl.when(i == H - 3)
            def _():
                zero_start(first, first + 56)
                ka[1 + (H + ring - 2) % ring, :, pl.ds(0, KEEP * DH), :] = keep[...]
        assert DEPTH == NSTEP
        _loop(0, H, layer3)
        _loop(last, first, lambda k: zero_copy(dkb_hbm, k, 1).wait())
        fill["waited"] = first

    def gradient_phases(late_tables, late_vectors, xout):
        tab.extend(late_tables.at[i] for i in range(late_tables.shape[0]))
        vec_at.extend((late_vectors, i) for i in range(late_vectors.shape[0]))
        zero_more(30)
        add_residual(woa, O3)
        normalise(N4, R4)
        to_heads(vec(N4), wqb, NN, Q4)
        zero_more(18)
        to_heads(vec(G4), wob, NT, DO4)
        zero_more(12)

        nbt = WIN // DH

        def layer4(g):
            q4, q2 = tab[Q4][grp(g), :], tab[Q2][grp(g), :]
            p = _softmax(b_scores(lambda r: _pair(q4, q2, r), kb, g) * SCALE)
            park_store(1, g * nbt, p.astype(BF16))
            p4 = p[:G, :]
            tab[O4][grp(g), :] = b_mix(p4, vb, g)
            do = tab[DO4][grp(g), :]
            dp = b_scores(lambda r: _only_row(do, r).astype(BF16), vb, g)
            ds = p4 * (dp - delta(O4, DO4, g)) * SCALE
            park_store(1, (NG + g) * nbt, jnp.concatenate([ds, ds], axis=0).astype(BF16))
            tab[DQ4][grp(g), :] = b_mix(ds, kb, g)
        loop_with_zeros(NG, 29, layer4)
        add_residual(wob, O4)
        xout[0] = vec(X)[0:1, :].astype(BF16)
        out_copy = pltpu.make_async_copy(xout.at[0], out_hbm, sem_vec.at[0])
        out_copy.start()
        put(G3, grad_below(wqb, DQ4, G4, N4, R4))
        zero_more(22)

        to_heads(vec(G3), woa, NT, DO3)
        apply_m(lambda h: ka[m3_at(h)], DO3, DQ3)
        zero_more(18)
        put(G2, grad_below(wqa, DQ3, G3, N3, R3))
        zero_more(14)

        to_heads(vec(G2), wob, NT, DO2)
        zero_more(12)

        def layer2_bwd(g):
            do = tab[DO2][grp(g), :]
            dp = b_scores(lambda r: _only_row(do, r).astype(BF16), vb, g)
            p2 = park_load(1, g * nbt, nbt).astype(F32)[G:, :]
            ds = p2 * (dp - delta(O2, DO2, g)) * SCALE
            ds4 = park_load(1, (NG + g) * nbt, nbt).astype(F32)[:G, :]
            park_store(1, (NG + g) * nbt, jnp.concatenate([ds4, ds], axis=0).astype(BF16))
            tab[DQ2][grp(g), :] = b_mix(ds, kb, g)
        loop_with_zeros(NG, 14, layer2_bwd)
        put(G1, grad_below(wqb, DQ2, G2, N2, R2))
        zero_more(14)

        to_heads(vec(G1), woa, NT, DO1)
        apply_m(lambda h: m1[h], DO1, DQ1)
        zero_more(18)
        xout[1] = grad_below(wqa, DQ1, G1, N1, R1)[0:1, :].astype(BF16)
        dx_copy = pltpu.make_async_copy(xout.at[1], dx_hbm, sem_vec.at[1])
        dx_copy.start()
        zero_more(24)

        def b_grads(i):
            g, c = i // (WIN // OC), i % (WIN // OC)
            rhs = outer_rhs(tab[DO4][grp(g), :], tab[DO2][grp(g), :], tab[Q4][grp(g), :], tab[Q2][grp(g), :])
            t0 = g * nbt + c * (OC // DH)
            at = jnp.concatenate([park_load(1, t0, OC // DH), park_load(1, NG * nbt + t0, OC // DH)], axis=0).T
            for r in range(G):
                vb[g * G + r, _ds(c * OC, OC), :] = _dot(at, rhs[r][0], NN).astype(BF16)
                kb[g * G + r, _ds(c * OC, OC), :] = _dot(at, rhs[r][1], NN).astype(BF16)
        loop_with_zeros(NG * WIN // OC, 8, b_grads)
        zero_more(2 * NZ - fill["issued"])

        def weight_grads(wq, wo, na, nb, dqa, dqb, oa, ob, ga, gb, which):
            unroll = 4
            per = NG * WIN // WR // (H // unroll)

            def db_start(k):
                g, row = k // (WIN // WR), k % (WIN // WR) * WR
                pltpu.make_async_copy(kvb.at[which, grp(g), _ds(row, WR), :],
                                      (dkb_hbm, dvb_hbm)[which].at[grp(g), _ds(SK - WIN + row, WR), :],
                                      sem_stage.at[which]).start()

            def body(i):
                _loop(i * per, (i + 1) * per, db_start)
                g, r0 = i // (G // unroll), i % (G // unroll) * unroll
                ns = jnp.concatenate([vec(na), vec(nb)], axis=0).astype(BF16).T
                gs = jnp.concatenate([vec(ga), vec(gb)], axis=0).astype(BF16)
                for k in range(unroll):
                    r = r0 + k
                    dq = _pair(tab[dqa][grp(g), :], tab[dqb][grp(g), :], r)
                    wq[:, :, _ds(g * GW + r * DH, DH)] = _dot(ns, dq, NN).astype(BF16).reshape(NS, D // NS, DH)
                    o = _pair(tab[oa][grp(g), :], tab[ob][grp(g), :], r)
                    wo[g, _ds(r * DH, DH), :] = _dot(o, gs, TN).astype(BF16)
            _loop(0, H // unroll, body)

        weight_grads(wqb, wob, N4, N2, DQ4, DQ2, O4, O2, G4, G2, 0)
        weight_grads(wqa, woa, N3, N1, DQ3, DQ1, O3, O1, G3, G1, 1)
        dw = ((wqa, dwqa_hbm), (wqb, dwqb_hbm), (woa, dwoa_hbm), (wob, dwob_hbm))

        def dw_start(view, first, j):
            for k in (first, first + 1):
                pltpu.make_async_copy(*view(*dw[k], j), sem_dw.at[k]).start()

        def staged_wait(k):
            stage = kvb.at[k % 2]
            pltpu.make_async_copy(stage, stage, sem_stage.at[k]).wait()

        def a_rows(i):
            return i // (QR // WR), _ds(i % (QR // WR) * WR, WR)

        def dv_start(g, i):
            idx = (grp(g),) + a_rows(i)
            pltpu.make_async_copy(va.at[idx], dva_hbm.at[idx], sem_dv.at[0]).start()

        def dk_start(g, i):
            part, rows = a_rows(i)
            pltpu.make_async_copy(kvb.at[g % 2, grp(part), rows], dka_hbm.at[grp(g), part, rows],
                                  sem_stage.at[2 + g]).start()

        def a_grads(g):
            staged_wait(g)
            gather_probs(g, 2)
            do3, do1 = tab[DO3][grp(g), :], tab[DO1][grp(g), :]
            rhs = outer_rhs(do3, do1, tab[Q3][grp(g), :], tab[Q1][grp(g), :])
            dl = jnp.concatenate([delta(O3, DO3, g), delta(O1, DO1, g)], axis=0)
            half = SK // OC // 2
            per = SK // WR // half

            def body(c):
                part, rows = c // (QR // OC), _ds(c % (QR // OC) * OC, OC)
                dp = _dot(_pair(do3, do1, 0), va[g * G, part, rows, :], NT)
                for r in range(1, G):
                    dp = dp + _dot(_pair(do3, do1, r), va[g * G + r, part, rows, :], NT)
                p = park_load(2, c * (OC // DH), OC // DH)
                ds = (p.astype(F32) * (dp - dl) * SCALE).astype(BF16)
                at = jnp.concatenate([p, ds], axis=0).T
                for r in range(G):
                    va[g * G + r, part, rows, :] = _dot(at, rhs[r][0], NN).astype(BF16)
                    kvb[g % 2, part * G + r, rows, :] = _dot(at, rhs[r][1], NN).astype(BF16)

                @pl.when(c >= half)
                def _():
                    _loop((c - half) * per, (c - half + 1) * per, lambda i: dv_start(g, i))

                @pl.when(jnp.logical_and(c < half, g > 0))
                def _():
                    _loop(c * per, (c + 1) * per, lambda i: dk_start(g - 1, i))

                @pl.when(jnp.logical_and(c < half // 2, g == 0))
                def _():
                    n = NWO // (half // 2)
                    _loop(c * n, (c + 1) * n, lambda j: dw_start(wo_view, 2, j))

                @pl.when(jnp.logical_and(c // (half // 2) == 1, g == 0))
                def _():
                    n = NWQ // (half // 2)
                    _loop((c - half // 2) * n, (c - half // 2 + 1) * n, lambda j: dw_start(wq_view, 0, j))
            _loop(0, SK // OC, body)
        _loop(0, NG, a_grads)
        _loop(0, SK // WR, lambda i: dk_start(NG - 1, i))

        _loop(fill["waited"], NZ, lambda i: zero_copy(dkb_hbm, i).wait())
        _loop(0, NZ, lambda i: zero_copy(dvb_hbm, i).wait())
        out_copy.wait()
        dx_copy.wait()
        for k, pair in enumerate(dw):
            pltpu.make_async_copy(*pair, sem_dw.at[k]).wait()
        pltpu.make_async_copy(va, dva_hbm, sem_dv.at[0]).wait()
        staged_wait(NG)
        staged_wait(NG + 1)

    pl.run_scoped(read_phases,
                  pltpu.VMEM((2 * SK // DH, DH), F32),
                  pltpu.VMEM((NS, KEEP * DH, DH), BF16),
                  pltpu.VMEM((2, 1, D), BF16))
    pl.run_scoped(gradient_phases,
                  pltpu.VMEM((16 - EARLY_TABLES, H, DH), F32),
                  pltpu.VMEM((13 - EARLY_VECTORS, D), F32),
                  pltpu.VMEM((2, 1, D), BF16))


@jax.jit
def pallas_interleave_layers__gqa_block_cached__sliding_block_cached__decode_kernel(
    A_x: jax.Array,
    A_k_cache: jax.Array,
    A_v_cache: jax.Array,
    A_wq: jax.Array,
    A_wo: jax.Array,
    B_x: jax.Array,
    B_k_cache: jax.Array,
    B_v_cache: jax.Array,
    B_wq: jax.Array,
    B_wo: jax.Array,
    grad_out: jax.Array,
):
    del B_x
    a_view = (H, NS, QR, DH)
    b_view = (H, SK, DH)
    wq_view = (NS, D // NS, H * DH)
    wo_view = (NG, GW, D)
    vec, a_out, b_out, wq, wo = (
        jax.ShapeDtypeStruct(s, BF16) for s in ((1, D), a_view, b_view, wq_view, wo_view))
    hbm = pl.BlockSpec(memory_space=pl.ANY)
    out, dx, dka, dva, dwqa, dwoa, dkb, dvb, dwqb, dwob = pl.pallas_call(
        _kernel,
        in_specs=[hbm] * 10,
        out_specs=[hbm] * 10,
        out_shape=[vec, vec, a_out, a_out, wq, wo, b_out, b_out, wq, wo],
        scratch_shapes=[
            pltpu.VMEM(a_view, BF16),
            pltpu.VMEM((2, H, WIN, DH), BF16),
            pltpu.VMEM((NSLOT, NS, QR, DH), BF16),
            pltpu.VMEM(wq_view, BF16),
            pltpu.VMEM(wo_view, BF16),
            pltpu.VMEM(wq_view, BF16),
            pltpu.VMEM(wo_view, BF16),
            pltpu.VMEM((H, DH, DH), BF16),
            pltpu.VMEM((G, ZR, DH), BF16),
            pltpu.VMEM((EARLY_TABLES, H, DH), F32),
            pltpu.VMEM((EARLY_VECTORS, D), F32),
            pltpu.SemaphoreType.DMA((DEPTH,)),
            pltpu.SemaphoreType.DMA((4,)),
            pltpu.SemaphoreType.DMA((2,)),
            pltpu.SemaphoreType.DMA((2,)),
            pltpu.SemaphoreType.DMA((2 + NG,)),
            pltpu.SemaphoreType.DMA((1,)),
        ],
        compiler_params=pltpu.CompilerParams(
            vmem_limit_bytes=128 * 1024 * 1024,
            disable_bounds_checks=True,
            flags={"XLA_TPU_FORCE_LP_LLO_SCHEDULER": True, "XLA_TPU_RESCHEDULE_DMA_DONES": True}),
    )(A_x.reshape(1, D), A_k_cache.reshape(a_view), A_v_cache.reshape(a_view),
      A_wq.reshape(wq_view), A_wo.reshape(wo_view),
      B_k_cache.reshape(b_view), B_v_cache.reshape(b_view),
      B_wq.reshape(wq_view), B_wo.reshape(wo_view), grad_out.reshape(1, D))
    return (out.reshape(A_x.shape), dx.reshape(A_x.shape),
            dka.reshape(A_k_cache.shape), dva.reshape(A_v_cache.shape),
            dwqa.reshape(A_wq.shape), dwoa.reshape(A_wo.shape),
            dkb.reshape(B_k_cache.shape), dvb.reshape(B_v_cache.shape),
            dwqb.reshape(B_wq.shape), dwob.reshape(B_wo.shape))
```

```python
import jax
import jax.numpy as jnp
from jax import lax
import jax.experimental.pallas as pl
import jax.experimental.pallas.tpu as pltpu

F32 = jnp.float32
BF16 = jnp.bfloat16

D = 640
H = 32
DH = 128
SK = 8192
WIN = 2048
EPS = 1e-5
SCALE = DH ** -0.5

G = 8
NG = H // G
GW = G * DH
NS = 4
QR = SK // NS
NSTEP = QR // DH
DEPTH = 16
NSLOT = 5
KEEP = 3
CH = 256
NCH = SK // CH
OC = 512
WR = 64
ZR = 64
WQ_ROWS, WQ_COLS = 8, 2048
WO_ROWS = 32
NWQ = D // NS // WQ_ROWS * (H * DH // WQ_COLS)
NWO = H * DH // NS // WO_ROWS
NZ = NG * (SK - WIN) // ZR

NN = (((1,), (0,)), ((), ()))
NT = (((1,), (1,)), ((), ()))
TN = (((0,), (0,)), ((), ()))

Q1, Q2, Q3, O1, O2, O3, Q4, O4, DO1, DO2, DO3, DO4, DQ1, DQ2, DQ3, DQ4 = range(16)
EARLY_TABLES = 6
X, N1, N2, N3, R1, R2, R3, G4, N4, R4, G1, G2, G3 = range(13)
EARLY_VECTORS = 8


def _dot(a, b, dims):
    return lax.dot_general(a, b, dims, preferred_element_type=F32)


def _row_ids():
    return lax.broadcasted_iota(jnp.int32, (G, DH), 0)


def _only_row(x, r):
    return jnp.where(_row_ids() == r, x, 0.0)


def _block_diag(x):
    return jnp.concatenate([_only_row(x, r) for r in range(G)], axis=1)


def _compact(y):
    out = y[:, :DH]
    for r in range(1, G):
        out = jnp.where(_row_ids() == r, y[:, r * DH:(r + 1) * DH], out)
    return out


def _pair(a, b, r):
    return jnp.concatenate([_only_row(a, r), _only_row(b, r)], axis=0).astype(BF16)


def _layernorm(x):
    mean = jnp.mean(x, axis=-1, keepdims=True)
    xc = x - mean
    var = jnp.mean(xc * xc, axis=-1, keepdims=True)
    rstd = 1.0 / jnp.sqrt(var + EPS)
    return xc * rstd, rstd


def _layernorm_bwd(dn, n, rstd):
    return rstd * (dn - jnp.mean(dn, axis=-1, keepdims=True)
                   - n * jnp.mean(dn * n, axis=-1, keepdims=True))


def _softmax(s):
    e = jnp.exp(s - jnp.max(s, axis=-1, keepdims=True))
    return e * (1.0 / jnp.sum(e, axis=-1, keepdims=True))


def _dense_softmax(tiles, span):
    def per_query(op, reduce, parts):
        v = parts[0]
        for part in parts[1:]:
            v = op(v, part)
        v = reduce(v, axis=1, keepdims=True)
        return jnp.concatenate(
            [jnp.broadcast_to(reduce(v[r:r + span], axis=0, keepdims=True), (span, 1))
             for r in range(0, G, span)], axis=0)
    tiles = [t * SCALE for t in tiles]
    top = per_query(jnp.maximum, jnp.max, tiles)
    e = [jnp.exp(t - top) for t in tiles]
    inv = 1.0 / per_query(jnp.add, jnp.sum, e)
    return jnp.concatenate([t * inv for t in e], axis=0)


def _ds(start, size):
    if isinstance(start, int):
        return pl.ds(start, size)
    return pl.ds(pl.multiple_of(start, size), size)


def _loop(lo, hi, body):
    def step(i, carry):
        body(i)
        return carry
    if not (isinstance(lo, int) and isinstance(hi, int)) or hi > lo:
        lax.fori_loop(lo, hi, step, 0)


def _kernel(x_hbm, ka_hbm, va_hbm, wqa_hbm, woa_hbm, kb_hbm, vb_hbm, wqb_hbm, wob_hbm, g_hbm,
            out_hbm, dx_hbm, dka_hbm, dva_hbm, dwqa_hbm, dwoa_hbm, dkb_hbm, dvb_hbm, dwqb_hbm, dwob_hbm,
            va, kvb, ka, wqa, woa, wqb, wob, m1, zeros, tables, vectors,
            sem_read, sem_dw, sem_vec, sem_zero, sem_stage, sem_dv):
    kb, vb = kvb.at[0], kvb.at[1]
    tab = [tables.at[i] for i in range(EARLY_TABLES)]
    vec_at = [(vectors, i) for i in range(EARLY_VECTORS)]

    def grp(g):
        return _ds(g * G, G)

    def step_start(view, n, urgent=True):
        src, dst = view
        sem = sem_read.at[n % DEPTH]
        slow = pl.ds(0, NS - 1)
        pltpu.make_async_copy(src.at[NS - 1], dst.at[NS - 1], sem).start(priority=0 if urgent else 1)
        pltpu.make_async_copy(src.at[slow], dst.at[slow], sem).start(priority=1)

    def step_wait(view, n):
        pltpu.make_async_copy(*view, sem_read.at[n % DEPTH]).wait()

    def wq_view(src, dst, j):
        per = H * DH // WQ_COLS
        idx = (slice(None), _ds(j // per * WQ_ROWS, WQ_ROWS), _ds(j % per * WQ_COLS, WQ_COLS))
        return src.at[idx], dst.at[idx]

    def wo_view(src, dst, j):
        idx = (slice(None), _ds(j * WO_ROWS, WO_ROWS), slice(None))
        return src.at[idx], dst.at[idx]

    def b_views(j):
        heads, c = _ds(j // (WIN // DH) * NS, NS), j % (WIN // DH)
        return [(src.at[heads, _ds(SK - WIN + c * DH, DH), :], dst.at[heads, _ds(c * DH, DH), :])
                for src, dst in ((kb_hbm, kb), (vb_hbm, vb))]

    def k_view(head, slot, c):
        rows = _ds(c * DH, DH)
        return ka_hbm.at[head, :, rows, :], ka.at[slot, :, rows, :]

    def v_view(head, c):
        rows = _ds(c * DH, DH)
        return va_hbm.at[head, :, rows, :], va.at[head, :, rows, :]

    def slot1(head):
        return (head + NSLOT - H % NSLOT) % NSLOT

    def pair_view(m, j):
        return k_view(m + 1, slot1(m + 1), j // 2) if j % 2 == 0 else v_view(m, j // 2)

    def zero_copy(dst, i, sem=0):
        per = NZ // NG
        return pltpu.make_async_copy(zeros, dst.at[grp(i // per), _ds(i % per * ZR, ZR), :], sem_zero.at[sem])

    def zero_start(lo, hi):
        if isinstance(lo, int):
            _loop(min(lo, NZ), min(hi, NZ), lambda i: zero_copy(dkb_hbm, i).start())
            _loop(max(lo, NZ) - NZ, max(hi, NZ) - NZ, lambda i: zero_copy(dvb_hbm, i).start())
        else:
            _loop(jnp.minimum(lo, NZ), jnp.minimum(hi, NZ), lambda i: zero_copy(dkb_hbm, i).start())
            _loop(jnp.maximum(lo, NZ) - NZ, jnp.maximum(hi, NZ) - NZ, lambda i: zero_copy(dvb_hbm, i).start())

    fill = {"issued": 0, "waited": 0}

    def take_zeros(n):
        fill["issued"] += n
        assert fill["issued"] <= 2 * NZ
        return fill["issued"] - n

    def zero_more(n):
        lo = take_zeros(n)
        zero_start(lo, lo + n)

    def loop_with_zeros(count, n, body):
        lo = take_zeros(count * n)

        def both(i):
            body(i)
            zero_start(lo + i * n, lo + (i + 1) * n)
        _loop(0, count, both)

    def vec(i):
        ref, row = vec_at[i]
        return jnp.broadcast_to(ref[row:row + 1, :], (G, D))

    def put(i, val):
        ref, row = vec_at[i]
        ref[row:row + 1, :] = jnp.broadcast_to(val, (G, D))[0:1, :]

    def weight(w, g):
        return w[g] if w.shape[-1] == D else w[:, :, _ds(g * GW, GW)].reshape(D, GW)

    def to_heads_group(vector, w, dims, dst, g):
        tab[dst][grp(g), :] = _compact(_dot(vector.astype(BF16), weight(w, g), dims))

    def to_heads(vector, w, dims, dst):
        _loop(0, NG, lambda g: to_heads_group(vector, w, dims, dst, g))

    def from_heads(src, w, dims):
        def body(g, acc):
            return acc + _dot(_block_diag(tab[src][grp(g), :]).astype(BF16), weight(w, g), dims)
        acc = lax.fori_loop(0, NG, body, jnp.zeros((G, D), F32))
        return jnp.broadcast_to(jnp.sum(acc, axis=0, keepdims=True), (G, D))

    def normalise(n, r):
        norm, rstd = _layernorm(vec(X))
        put(n, norm)
        put(r, rstd)

    def add_residual(wo, o):
        put(X, vec(X) + from_heads(o, wo, NN))

    def grad_below(wq, dq, g, n, r):
        return vec(g) + _layernorm_bwd(from_heads(dq, wq, NT), vec(n), vec(r))

    def delta(o, do, g):
        return jnp.sum(tab[o][grp(g), :] * tab[do][grp(g), :], axis=1, keepdims=True)

    def head_row(t, head):
        return jnp.broadcast_to(tab[t][pl.ds(head, 1), :], (G, DH))

    def chunk(ref, i, c):
        return ref[i, c // (QR // CH), pl.ds(c % (QR // CH) * CH, CH), :]

    def add_scores(s, q, span, slot, c):
        y = _dot(q, chunk(ka, slot, c), NT)
        for t in range(CH // DH):
            r = (c * (CH // DH) + t) % span
            tile = y[:, t * DH:(t + 1) * DH]
            if r == 0:
                s.append(tile)
            else:
                s[-1] = jnp.where(_row_ids() % span == r, tile, s[-1])

    def first_probs(probs, q, span, slot):
        s = []
        for c in range(NCH):
            add_scores(s, q.astype(BF16), span, slot, c)
        probs[pl.ds(0, len(s) * G), :] = _dense_softmax(s, span)

    def a_head(probs, span, slot, head, q_next, slot_next, dma):
        qb = q_next.astype(BF16)
        acc = jnp.zeros((DH + 16, DH), F32)
        ksum = jnp.zeros((DH, DH), F32)
        s = []
        for c in range(NCH):
            if c % 2 == 0:
                dma(c // 2)
            add_scores(s, qb, span, slot_next, c)
            p = jnp.concatenate(
                [jnp.broadcast_to(probs[pl.ds(t // span * G + t % span, 1), :], (G, DH))
                 for t in range(c * (CH // DH), (c + 1) * (CH // DH))], axis=1)
            kp = chunk(ka, slot, c).T.astype(F32) * jnp.concatenate([p] * (DH // G), axis=0)
            for t in range(CH // DH):
                ksum = ksum + kp[:, t * DH:(t + 1) * DH]
            lhs = jnp.concatenate([kp, p, p], axis=0).astype(BF16)
            acc = acc + _dot(lhs, chunk(va, head, c), NN)
        o = acc[DH:DH + 1, :]
        kbar = jnp.sum(ksum, axis=1, keepdims=True)
        return o, (acc[:DH, :] - kbar * o).astype(BF16), _dense_softmax(s, span)

    def apply_m(m_of_head, src, dst):
        def body(g):
            do = tab[src][grp(g), :]
            dq = jnp.zeros((G, DH), F32)
            for r in range(G):
                dq = dq + _dot(_only_row(do, r).astype(BF16), m_of_head(g * G + r), NT)
            tab[dst][grp(g), :] = dq * SCALE
        _loop(0, NG, body)

    def p_at(head, row0=0, rows=DH):
        return 0, head // NSTEP, _ds(head % NSTEP * DH + row0, rows), slice(None)

    def m3_at(head):
        return 0, NS // 2 + head // NSTEP, _ds(head % NSTEP * DH, DH), slice(None)

    def park_load(slot, tile0, n):
        val = ka[slot, 0, _ds(tile0 * 16, n * 16), :]
        return jnp.concatenate([val[t * 16:(t + 1) * 16, :] for t in range(n)], axis=1)

    def park_store(slot, tile0, val):
        n = val.shape[1] // DH
        ka[slot, 0, _ds(tile0 * 16, n * 16), :] = jnp.concatenate(
            [val[:, t * DH:(t + 1) * DH] for t in range(n)], axis=0)

    def gather_probs(g, slot):
        span, rows = G // 2, 32

        def body(i):
            src = [ka[p_at(g * G + r, i * rows, rows)].astype(F32) for r in range(G)]
            tiles = []
            for t in range(rows // G * span):
                halves = []
                for k in range(2):
                    j = t // span * G + k * span + t % span
                    out = jnp.broadcast_to(src[0][j:j + 1, :], (G, DH))
                    for r in range(1, G):
                        out = jnp.where(_row_ids() == r, jnp.broadcast_to(src[r][j:j + 1, :], (G, DH)), out)
                    halves.append(out)
                tiles.append(jnp.concatenate(halves, axis=0).astype(BF16))
            park_store(slot, i * len(tiles), jnp.concatenate(tiles, axis=1))
        _loop(0, DH // rows, body)

    def b_scores(lhs_of_row, ref, g):
        s = _dot(lhs_of_row(0), ref[g * G], NT)
        for r in range(1, G):
            s = s + _dot(lhs_of_row(r), ref[g * G + r], NT)
        return s

    def b_mix(p, ref, g):
        pb = p.astype(BF16)
        out = _dot(pb, ref[g * G], NN)
        for r in range(1, G):
            out = jnp.where(_row_ids() == r, _dot(pb, ref[g * G + r], NN), out)
        return out

    def outer_rhs(do_a, do_b, q_a, q_b):
        zero = jnp.zeros((16, DH), BF16)
        return [(jnp.concatenate([_pair(do_a, do_b, r), zero], axis=0),
                 jnp.concatenate([zero, _pair(q_a, q_b, r)], axis=0)) for r in range(G)]

    def read_phases(probs, keep, xin):
        x_copy = pltpu.make_async_copy(x_hbm, xin.at[0], sem_vec.at[0])
        g_copy = pltpu.make_async_copy(g_hbm, xin.at[1], sem_vec.at[1])

        segments = [
            (NWQ, lambda j: [wq_view(wqa_hbm, wqa, j), wq_view(wqb_hbm, wqb, j)]),
            (NWO, lambda j: [wo_view(woa_hbm, woa, j), wo_view(wob_hbm, wob, j)]),
            (H // NS * (WIN // DH), b_views),
        ]
        lead_in = [k_view(0, slot1(0), c) for c in range(NSTEP)]
        lead_in += [pair_view(m, j) for m in range(2) for j in range(2 * NSTEP)]
        lag = DEPTH // 2
        for j in range(lag):
            for k, view in enumerate(segments[0][1](j)):
                step_start(view, 2 * j + k, urgent=False)
            if j == 0:
                x_copy.start()
                g_copy.start()
        zeros[...] = jnp.zeros(zeros.shape, BF16)
        for si, (count, views) in enumerate(segments):
            assert count % lag == 0

            def advance(j, ahead, views=views):
                for k, (old, new) in enumerate(zip(views(j), ahead)):
                    step_wait(old, 2 * j + k)
                    step_start(new, 2 * j + k)

            def most(j, si=si, views=views, advance=advance):
                advance(j, views(j + lag))
                if si == 2:
                    pl.when(jnp.logical_and(j % G == G - 1, j < NG * G))(
                        lambda: to_heads_group(vec(N1), wqa, NN, Q1, j // G))
            _loop(0, count - lag, most)
            if si + 1 < len(segments):
                _loop(count - lag, count, lambda j, nxt=segments[si + 1][1], advance=advance, count=count:
                      advance(j, nxt(j + lag - count)))
            else:
                for j in range(count - lag, count):
                    advance(j, lead_in[2 * (j + lag - count):][:2])
            if si == 1:
                x_copy.wait()
                g_copy.wait()
                put(X, xin[0].astype(F32))
                put(G4, xin[1].astype(F32))
                normalise(N1, R1)
        for n in range(3 * NSTEP):
            step_wait(lead_in[n], n)
            step_start(lead_in[n + DEPTH], n)

        first_probs(probs, head_row(Q1, 0), G, slot1(0))
        kept = H - NSLOT - 1
        first = take_zeros(64)

        def layer1(h):
            def dma(i):
                for j in (2 * i, 2 * i + 1):
                    pl.when(h + 2 < H)(lambda: step_wait(pair_view(h + 1, j), j))
                    m, k = h + 1 + (j + DEPTH) // (2 * NSTEP), (j + DEPTH) % (2 * NSTEP)
                    pl.when(m + 1 - k % 2 < H)(lambda: step_start(pair_view(m, k), j))

            nxt = jnp.minimum(h + 1, H - 1)
            o, m, p = a_head(probs, G, slot1(h), h, head_row(Q1, nxt), slot1(nxt), dma)
            m1[h] = m
            tab[O1][pl.ds(h, 1), :] = o
            probs[pl.ds(0, SK // DH), :] = p

            @pl.when(h == kept)
            def _():
                keep[...] = ka[slot1(kept), :, pl.ds(0, KEEP * DH), :]

            @pl.when(h == H - 2)
            def _():
                zero_start(first, first + 64)
                for j in range(1, 2 * NSTEP, 2):
                    step_wait(pair_view(H - 1, j), j)
        _loop(0, H, layer1)
        zero_more(13)
        add_residual(woa, O1)
        normalise(N2, R2)
        to_heads(vec(N2), wqb, NN, Q2)
        zero_more(18)

        def layer2(g):
            q = tab[Q2][grp(g), :]
            p = _softmax(b_scores(lambda r: _only_row(q, r).astype(BF16), kb, g) * SCALE)
            tab[O2][grp(g), :] = b_mix(p, vb, g)
        loop_with_zeros(NG, 15, layer2)
        add_residual(wob, O2)
        normalise(N3, R3)
        to_heads(vec(N3), wqa, NN, Q3)
        zero_more(4)
        between_reads = fill["issued"]
        last = take_zeros(1)
        zero_copy(dkb_hbm, last, 1).start()

        ring = NSLOT - 1
        first = take_zeros(64)
        more = take_zeros(26)
        assert first <= NZ

        def head3(i):
            return (i + H - NSLOT) % H

        def slot3(i):
            return jnp.where(i == 0, 0, 1 + (i + ring - 1) % ring)

        def queries(head):
            return jnp.where(_row_ids() < G // 2, head_row(Q3, head), head_row(Q1, head))

        first_probs(probs, queries(head3(0)), G // 2, 0)

        def layer3(i):
            def dma(c):
                pl.when(jnp.logical_and(i + 2 >= NSLOT, i + 2 < H - 1))(
                    lambda: step_wait(k_view(head3(i + 2), slot3(i + 2), c), c))
                pl.when(jnp.logical_and(i + 3 >= NSLOT, i + 3 < (H - 1 if c < KEEP else H)))(
                    lambda: step_start(k_view(head3(i + 3), slot3(i + 3), c), c))

            @pl.when(i == NSLOT - 3)
            def _():
                _loop(0, between_reads, lambda k: zero_copy(dkb_hbm, k).wait())

            head, nxt = head3(i), jnp.minimum(i + 1, H - 1)
            o, m, p = a_head(probs, G // 2, slot3(i), head, queries(head3(nxt)), slot3(nxt), dma)
            ka[m3_at(head)] = m
            tab[O3][pl.ds(head, 1), :] = o
            ka[p_at(head)] = probs[...].astype(BF16)
            probs[...] = p

            @pl.when(i == H - 4)
            def _():
                slot = 1 + (H + ring - 2) % ring
                ka[slot, :, pl.ds(0, KEEP * DH), :] = keep[...]
                for c in range(KEEP, NSTEP):
                    if c == NSTEP - 5:
                        zero_start(first, first + 64)
                    step_wait(k_view(kept, slot, c), c)
            pl.when(jnp.logical_and(i > H - 4, i < H - 1))(
                lambda: zero_start(more + (i - H + 3) * 13, more + (i - H + 4) * 13))
        assert DEPTH == NSTEP
        _loop(0, H, layer3)
        zero_copy(dkb_hbm, last, 1).wait()
        fill["waited"] = first

    def gradient_phases(late_tables, late_vectors, xout):
        tab.extend(late_tables.at[i] for i in range(late_tables.shape[0]))
        vec_at.extend((late_vectors, i) for i in range(late_vectors.shape[0]))
        zero_more(13)
        add_residual(woa, O3)
        normalise(N4, R4)
        to_heads(vec(N4), wqb, NN, Q4)
        zero_more(18)
        to_heads(vec(G4), wob, NT, DO4)
        zero_more(12)

        nbt = WIN // DH

        def layer4(g):
            q4, q2 = tab[Q4][grp(g), :], tab[Q2][grp(g), :]
            p = _softmax(b_scores(lambda r: _pair(q4, q2, r), kb, g) * SCALE)
            park_store(1, g * nbt, p.astype(BF16))
            p4 = p[:G, :]
            tab[O4][grp(g), :] = b_mix(p4, vb, g)
            do = tab[DO4][grp(g), :]
            dp = b_scores(lambda r: _only_row(do, r).astype(BF16), vb, g)
            ds = p4 * (dp - delta(O4, DO4, g)) * SCALE
            park_store(1, (NG + g) * nbt, jnp.concatenate([ds, ds], axis=0).astype(BF16))
            tab[DQ4][grp(g), :] = b_mix(ds, kb, g)
        loop_with_zeros(NG, 29, layer4)
        add_residual(wob, O4)
        xout[0] = vec(X)[0:1, :].astype(BF16)
        out_copy = pltpu.make_async_copy(xout.at[0], out_hbm, sem_vec.at[0])
        out_copy.start()
        put(G3, grad_below(wqb, DQ4, G4, N4, R4))
        zero_more(22)

        to_heads(vec(G3), woa, NT, DO3)
        apply_m(lambda h: ka[m3_at(h)], DO3, DQ3)
        zero_more(18)
        put(G2, grad_below(wqa, DQ3, G3, N3, R3))
        zero_more(14)

        to_heads(vec(G2), wob, NT, DO2)
        zero_more(12)

        def layer2_bwd(g):
            do = tab[DO2][grp(g), :]
            dp = b_scores(lambda r: _only_row(do, r).astype(BF16), vb, g)
            p2 = park_load(1, g * nbt, nbt).astype(F32)[G:, :]
            ds = p2 * (dp - delta(O2, DO2, g)) * SCALE
            ds4 = park_load(1, (NG + g) * nbt, nbt).astype(F32)[:G, :]
            park_store(1, (NG + g) * nbt, jnp.concatenate([ds4, ds], axis=0).astype(BF16))
            tab[DQ2][grp(g), :] = b_mix(ds, kb, g)
        loop_with_zeros(NG, 14, layer2_bwd)
        put(G1, grad_below(wqb, DQ2, G2, N2, R2))
        zero_more(14)

        to_heads(vec(G1), woa, NT, DO1)
        apply_m(lambda h: m1[h], DO1, DQ1)
        zero_more(18)
        xout[1] = grad_below(wqa, DQ1, G1, N1, R1)[0:1, :].astype(BF16)
        dx_copy = pltpu.make_async_copy(xout.at[1], dx_hbm, sem_vec.at[1])
        dx_copy.start()
        zero_more(24)

        def b_grads(i):
            g, c = i // (WIN // OC), i % (WIN // OC)
            rhs = outer_rhs(tab[DO4][grp(g), :], tab[DO2][grp(g), :], tab[Q4][grp(g), :], tab[Q2][grp(g), :])
            t0 = g * nbt + c * (OC // DH)
            at = jnp.concatenate([park_load(1, t0, OC // DH), park_load(1, NG * nbt + t0, OC // DH)], axis=0).T
            for r in range(G):
                vb[g * G + r, _ds(c * OC, OC), :] = _dot(at, rhs[r][0], NN).astype(BF16)
                kb[g * G + r, _ds(c * OC, OC), :] = _dot(at, rhs[r][1], NN).astype(BF16)
        loop_with_zeros(NG * WIN // OC, 8, b_grads)
        zero_more(2 * NZ - fill["issued"])

        def weight_grads(wq, wo, na, nb, dqa, dqb, oa, ob, ga, gb, which):
            unroll = 4
            per = NG * WIN // WR // (H // unroll)

            def db_start(k):
                g, row = k // (WIN // WR), k % (WIN // WR) * WR
                pltpu.make_async_copy(kvb.at[which, grp(g), _ds(row, WR), :],
                                      (dkb_hbm, dvb_hbm)[which].at[grp(g), _ds(SK - WIN + row, WR), :],
                                      sem_stage.at[which]).start()

            def body(i):
                _loop(i * per, (i + 1) * per, db_start)
                g, r0 = i // (G // unroll), i % (G // unroll) * unroll
                ns = jnp.concatenate([vec(na), vec(nb)], axis=0).astype(BF16).T
                gs = jnp.concatenate([vec(ga), vec(gb)], axis=0).astype(BF16)
                for k in range(unroll):
                    r = r0 + k
                    dq = _pair(tab[dqa][grp(g), :], tab[dqb][grp(g), :], r)
                    wq[:, :, _ds(g * GW + r * DH, DH)] = _dot(ns, dq, NN).astype(BF16).reshape(NS, D // NS, DH)
                    o = _pair(tab[oa][grp(g), :], tab[ob][grp(g), :], r)
                    wo[g, _ds(r * DH, DH), :] = _dot(o, gs, TN).astype(BF16)
            _loop(0, H // unroll, body)

        weight_grads(wqb, wob, N4, N2, DQ4, DQ2, O4, O2, G4, G2, 0)
        weight_grads(wqa, woa, N3, N1, DQ3, DQ1, O3, O1, G3, G1, 1)
        dw = ((wqa, dwqa_hbm), (wqb, dwqb_hbm), (woa, dwoa_hbm), (wob, dwob_hbm))

        def dw_start(view, first, j):
            for k in (first, first + 1):
                pltpu.make_async_copy(*view(*dw[k], j), sem_dw.at[k]).start()

        def staged_wait(k):
            stage = kvb.at[k % 2]
            pltpu.make_async_copy(stage, stage, sem_stage.at[k]).wait()

        def a_rows(i):
            return i // (QR // WR), _ds(i % (QR // WR) * WR, WR)

        def dv_start(g, i):
            idx = (grp(g),) + a_rows(i)
            pltpu.make_async_copy(va.at[idx], dva_hbm.at[idx], sem_dv.at[0]).start()

        def dk_start(g, i):
            part, rows = a_rows(i)
            pltpu.make_async_copy(kvb.at[g % 2, grp(part), rows], dka_hbm.at[grp(g), part, rows],
                                  sem_stage.at[2 + g]).start()

        def a_grads(g):
            staged_wait(g)
            gather_probs(g, 2)
            do3, do1 = tab[DO3][grp(g), :], tab[DO1][grp(g), :]
            rhs = outer_rhs(do3, do1, tab[Q3][grp(g), :], tab[Q1][grp(g), :])
            dl = jnp.concatenate([delta(O3, DO3, g), delta(O1, DO1, g)], axis=0)
            half = SK // OC // 2
            per = SK // WR // half

            def body(c):
                part, rows = c // (QR // OC), _ds(c % (QR // OC) * OC, OC)
                dp = _dot(_pair(do3, do1, 0), va[g * G, part, rows, :], NT)
                for r in range(1, G):
                    dp = dp + _dot(_pair(do3, do1, r), va[g * G + r, part, rows, :], NT)
                p = park_load(2, c * (OC // DH), OC // DH)
                ds = (p.astype(F32) * (dp - dl) * SCALE).astype(BF16)
                at = jnp.concatenate([p, ds], axis=0).T
                for r in range(G):
                    va[g * G + r, part, rows, :] = _dot(at, rhs[r][0], NN).astype(BF16)
                    kvb[g % 2, part * G + r, rows, :] = _dot(at, rhs[r][1], NN).astype(BF16)

                @pl.when(c >= half)
                def _():
                    _loop((c - half) * per, (c - half + 1) * per, lambda i: dv_start(g, i))

                @pl.when(jnp.logical_and(c < half, g > 0))
                def _():
                    _loop(c * per, (c + 1) * per, lambda i: dk_start(g - 1, i))

                @pl.when(jnp.logical_and(c < half // 2, g == 0))
                def _():
                    n = NWO // (half // 2)
                    _loop(c * n, (c + 1) * n, lambda j: dw_start(wo_view, 2, j))

                @pl.when(jnp.logical_and(c // (half // 2) == 1, g == 0))
                def _():
                    n = NWQ // (half // 2)
                    _loop((c - half // 2) * n, (c - half // 2 + 1) * n, lambda j: dw_start(wq_view, 0, j))
            _loop(0, SK // OC, body)
        _loop(0, NG, a_grads)
        _loop(0, SK // WR, lambda i: dk_start(NG - 1, i))

        _loop(fill["waited"], NZ, lambda i: zero_copy(dkb_hbm, i).wait())
        _loop(0, NZ, lambda i: zero_copy(dvb_hbm, i).wait())
        out_copy.wait()
        dx_copy.wait()
        for k, pair in enumerate(dw):
            pltpu.make_async_copy(*pair, sem_dw.at[k]).wait()
        pltpu.make_async_copy(va, dva_hbm, sem_dv.at[0]).wait()
        staged_wait(NG)
        staged_wait(NG + 1)

    pl.run_scoped(read_phases,
                  pltpu.VMEM((2 * SK // DH, DH), F32),
                  pltpu.VMEM((NS, KEEP * DH, DH), BF16),
                  pltpu.VMEM((2, 1, D), BF16))
    pl.run_scoped(gradient_phases,
                  pltpu.VMEM((16 - EARLY_TABLES, H, DH), F32),
                  pltpu.VMEM((13 - EARLY_VECTORS, D), F32),
                  pltpu.VMEM((2, 1, D), BF16))


@jax.jit
def pallas_interleave_layers__gqa_block_cached__sliding_block_cached__decode_kernel(
    A_x: jax.Array,
    A_k_cache: jax.Array,
    A_v_cache: jax.Array,
    A_wq: jax.Array,
    A_wo: jax.Array,
    B_x: jax.Array,
    B_k_cache: jax.Array,
    B_v_cache: jax.Array,
    B_wq: jax.Array,
    B_wo: jax.Array,
    grad_out: jax.Array,
):
    del B_x
    a_view = (H, NS, QR, DH)
    b_view = (H, SK, DH)
    wq_view = (NS, D // NS, H * DH)
    wo_view = (NG, GW, D)
    vec, a_out, b_out, wq, wo = (
        jax.ShapeDtypeStruct(s, BF16) for s in ((1, D), a_view, b_view, wq_view, wo_view))
    hbm = pl.BlockSpec(memory_space=pl.ANY)
    out, dx, dka, dva, dwqa, dwoa, dkb, dvb, dwqb, dwob = pl.pallas_call(
        _kernel,
        in_specs=[hbm] * 10,
        out_specs=[hbm] * 10,
        out_shape=[vec, vec, a_out, a_out, wq, wo, b_out, b_out, wq, wo],
        scratch_shapes=[
            pltpu.VMEM(a_view, BF16),
            pltpu.VMEM((2, H, WIN, DH), BF16),
            pltpu.VMEM((NSLOT, NS, QR, DH), BF16),
            pltpu.VMEM(wq_view, BF16),
            pltpu.VMEM(wo_view, BF16),
            pltpu.VMEM(wq_view, BF16),
            pltpu.VMEM(wo_view, BF16),
            pltpu.VMEM((H, DH, DH), BF16),
            pltpu.VMEM((G, ZR, DH), BF16),
            pltpu.VMEM((EARLY_TABLES, H, DH), F32),
            pltpu.VMEM((EARLY_VECTORS, D), F32),
            pltpu.SemaphoreType.DMA((DEPTH,)),
            pltpu.SemaphoreType.DMA((4,)),
            pltpu.SemaphoreType.DMA((2,)),
            pltpu.SemaphoreType.DMA((2,)),
            pltpu.SemaphoreType.DMA((2 + NG,)),
            pltpu.SemaphoreType.DMA((1,)),
        ],
        compiler_params=pltpu.CompilerParams(
            vmem_limit_bytes=128 * 1024 * 1024,
            disable_bounds_checks=True,
            flags={"XLA_TPU_FORCE_LP_LLO_SCHEDULER": True, "XLA_TPU_RESCHEDULE_DMA_DONES": True}),
    )(A_x.reshape(1, D), A_k_cache.reshape(a_view), A_v_cache.reshape(a_view),
      A_wq.reshape(wq_view), A_wo.reshape(wo_view),
      B_k_cache.reshape(b_view), B_v_cache.reshape(b_view),
      B_wq.reshape(wq_view), B_wo.reshape(wo_view), grad_out.reshape(1, D))
    return (out.reshape(A_x.shape), dx.reshape(A_x.shape),
            dka.reshape(A_k_cache.shape), dva.reshape(A_v_cache.shape),
            dwqa.reshape(A_wq.shape), dwoa.reshape(A_wo.shape),
            dkb.reshape(B_k_cache.shape), dvb.reshape(B_v_cache.shape),
            dwqb.reshape(B_wq.shape), dwob.reshape(B_wo.shape))
```
